```python
import jax
import jax.numpy as jnp

def _softmax(x, axis=-1):
    return jax.nn.softmax(x, axis=axis)

def _gelu(x):
    return jax.nn.gelu(x, approximate=True)

def _silu(x):
    return jax.nn.silu(x)

def _sigmoid(x):
    return jax.nn.sigmoid(x)

def _layernorm(x, axis=-1, eps=1e-05):
    m = jnp.mean(x, axis=axis, keepdims=True)
    v = jnp.var(x, axis=axis, keepdims=True)
    return (x - m) / jnp.sqrt(v + eps)

def _scatter_add(tgt, idx, src, axis=0):
    return tgt.at[idx].add(src)

def _segment_sum(src, seg, n):
    return jax.ops.segment_sum(src, seg, n)

class _Rng:

    def __init__(self, key):
        self._k = key

    def _next(self):
        self._k, sub = jax.random.split(self._k)
        return sub

    def normal(self, shape):
        return jax.random.normal(self._next(), shape, dtype=jnp.bfloat16)

    def randint(self, lo, hi, shape):
        return jax.random.randint(self._next(), shape, lo, hi, dtype=jnp.int32)

    def uniform(self, shape, lo=0.0, hi=1.0):
        return jax.random.uniform(self._next(), shape, jnp.bfloat16, lo, hi)

    def permutation(self, n):
        return jax.random.permutation(self._next(), n)
kernel_name = 'adaLN_cond__ssm_conv_h3__glu_gated_swiglu__prompt'

def setup_inputs():
    _rng = _Rng(jax.random.key(int.from_bytes(__import__("os").urandom(4), "little")))
    _w = lambda a: (lambda t: t.astype(jnp.bfloat16) if jnp.issubdtype(t.dtype, jnp.floating) else t)(jnp.asarray(a))

    def _A_setup():
        B, S, D = (1, 2048, 640)
        ks = 4
        return {'q': _w((lambda *s: _rng.normal(s) * 0.05)(B, S, D)), 'k': _w((lambda *s: _rng.normal(s) * 0.05)(B, S, D)), 'v': _w((lambda *s: _rng.normal(s) * 0.05)(B, S, D)), 'shift_k': _w((lambda *s: _rng.normal(s) * 0.05)(D, ks) * 0.5), 'ssm_k': _w((lambda *s: _rng.normal(s) * 0.05)(D, S) * (1.0 / S ** 0.5)), 'ssm_D': _w((lambda *s: _rng.normal(s) * 0.05)(D))}
    _A_in = _A_setup()

    def _B_setup():
        B, S, D, F = (1, 2048, 640, 1536)
        return {'x': _w((lambda *s: _rng.normal(s) * 0.05)(B, S, D)), 'w1': _w((lambda *s: _rng.normal(s) * 0.05)(D, F) * (2.0 / D) ** 0.5), 'w3': _w((lambda *s: _rng.normal(s) * 0.05)(D, F) * (2.0 / D) ** 0.5), 'w2': _w((lambda *s: _rng.normal(s) * 0.05)(F, D) * (2.0 / F) ** 0.5)}
    _B_in = _B_setup()
    return {'A_q': _A_in['q'], 'A_k': _A_in['k'], 'A_v': _A_in['v'], 'A_shift_k': _A_in['shift_k'], 'A_ssm_k': _A_in['ssm_k'], 'A_ssm_D': _A_in['ssm_D'], 'B_x': _B_in['x'], 'B_w1': _B_in['w1'], 'B_w3': _B_in['w3'], 'B_w2': _B_in['w2'], 'c': _w((lambda *s: _rng.normal(s) * 0.05)(1, 640)), 'w_mod': _w((lambda *s: _rng.normal(s) * 0.05)(640, 6 * 640) * 640 ** (-0.5))}

def reference(A_q, A_k, A_v, A_shift_k, A_ssm_k, A_ssm_D, B_x, B_w1, B_w3, B_w2, c, w_mod):

    def _A_ref(q, k, v, shift_k, ssm_k, ssm_D):
        B, S, D = q.shape
        ks = shift_k.shape[-1]
        k_pad = jnp.pad(k, ((0, 0), (ks - 1, 0), (0, 0)))
        k_shift = jnp.zeros_like(k)
        for t in range(ks):
            k_shift = k_shift + k_pad[:, t:t + S, :] * shift_k[:, ks - 1 - t][None, None, :]
        kv = k_shift * v
        L = 2 * S
        kv_pad = jnp.pad(kv, ((0, 0), (0, S), (0, 0)))
        kf_pad = jnp.pad(ssm_k, ((0, 0), (0, S)))
        kv_f = (lambda x, axes=(-2, -1): jnp.fft.rfft2(x.astype(jnp.float32), axes=axes))(kv_pad[:, None, :, :], axes=(1, 2))
        kf_f = (lambda x, axes=(-2, -1): jnp.fft.rfft2(x.astype(jnp.float32), axes=axes))(kf_pad[:, None, :], axes=(1, 2))
        kf_f = (lambda x, *d: x.transpose(*d))(kf_f, 1, 2, 0)
        y_f = kv_f * kf_f[None, :, :, :]
        y = (lambda x, s, axes=(-2, -1): jnp.fft.irfft2(x, s=s, axes=axes).astype(jnp.bfloat16))(y_f, (1, L), axes=(1, 2))[:, 0, :S, :]
        y = y + kv * ssm_D[None, None, :]
        return q * y

    def _B_ref(x, w1, w3, w2):
        gate = jnp.einsum('bsd,df->bsf', x, w1)
        up = jnp.einsum('bsd,df->bsf', x, w3)
        h = _silu(gate) * up
        out = jnp.einsum('bsf,fd->bsd', h, w2)
        return out
    x = A_q
    mod = (_silu(c) @ w_mod).reshape(c.shape[0], 6, 1, -1)
    sa, ca, ga, sb, cb, gb = (mod[:, 0].copy(), mod[:, 1].copy(), mod[:, 2].copy(), mod[:, 3].copy(), mod[:, 4].copy(), mod[:, 5].copy())
    h = _layernorm(x, axis=-1) * (1 + ca) + sa
    x = x + ga * _A_ref(h, A_k, A_v, A_shift_k, A_ssm_k, A_ssm_D)
    h = _layernorm(x, axis=-1) * (1 + cb) + sb
    x = x + gb * _B_ref(h, B_w1, B_w3, B_w2)
    return x
```

```python
import functools
import numpy as np
import jax
import jax.numpy as jnp
from jax import lax
import jax.experimental.pallas as pl
import jax.experimental.pallas.tpu as pltpu

S, D, F = 2048, 640, 1536
LANES = 128
NT = D // LANES
C = 256
NCH = S // C
T_OFF = 2 * NCH * 96
F_OFF = T_OFF + 2 * NCH * 16
G_OFF = F_OFF + 32
Z_ROWS = G_OFF + 32
BF, F32, U32 = jnp.bfloat16, jnp.float32, jnp.uint32


def _dft_consts():
    L = 2 * C
    f0 = np.concatenate([np.arange(0, 128, 2), np.arange(1, 128, 2)])
    a = np.arange(128)
    fm = np.zeros((2, 256, 128), np.float32)
    gm = np.zeros((2, 128, 256), np.float32)
    for p in range(2):
        th = 2 * np.pi * np.outer(f0 + 0.5, 2 * a + p) / L
        fm[p] = np.stack([np.cos(th).reshape(16, 8, 128), -np.sin(th).reshape(16, 8, 128)], axis=1).reshape(256, 128)
        gm[p, :, 0::2] = (2 / L) * np.cos(th).T
        gm[p, :, 1::2] = -(2 / L) * np.sin(th).T
    return fm.astype(BF), gm.astype(BF)


def _unpack(w, i):
    return pltpu.unpack_elementwise(w, index=i, packed_dtype=BF, unpacked_dtype=F32)


def _pack(lo, hi):
    return pltpu.pack_elementwise([lo, hi], packed_dtype=BF)


def _dot(a, b):
    return jnp.dot(a, b, preferred_element_type=F32)


def _causal_conv(x, k):
    n = len(x)
    out = []
    for i in range(n):
        acc = x[i] * k[0]
        for j in range(1, i + 1):
            acc = acc + x[i - j] * k[j]
        out.append(acc)
    return out


def _layernorm(x):
    m = jnp.mean(x, axis=-1, keepdims=True)
    xc = x - m
    v = jnp.mean(xc * xc, axis=-1, keepdims=True)
    return xc * lax.rsqrt(v + 1e-5)


def make(TM=256, FC=512, do_conv=True, do_ffn=True, flags=None, ORDER='ckGbGbGbGFbFbFbFbFbFbFtFbbbYX', UNROLL=1):
    NB = S // TM
    NFC = F // FC

    def body(q_hbm, k_hbm, v_hbm, shift_ref, s_hbm, d_ref, w1_hbm, w3_hbm, w2_hbm, c_ref, wm_hbm,
             fm_ref, gm_ref, o_hbm,
             kbuf, vbuf, sbuf, qbuf, w1buf, w3buf, w2buf, wmbuf, ybuf, obuf,
             xs0, xs1, ks0, ks1, zb, taps, mod, x1a, x1b, h2a, h2b,
             sem_in, sem_wm, sem_q, sem_w, sem_o):

        def conv_copies(t):
            cols = pl.ds(t * LANES, LANES)
            return [
                pltpu.make_async_copy(k_hbm.at[0, :, cols], kbuf.at[t, pl.ds(16, S), :], sem_in.at[1, t]),
                pltpu.make_async_copy(v_hbm.at[0, :, cols], vbuf.at[t], sem_in.at[2, t]),
            ]

        def s_copy(t):
            return pltpu.make_async_copy(s_hbm.at[pl.ds(t * LANES, LANES), :], sbuf.at[t], sem_in.at[0, t])

        def wm_copy(j):
            cols = pl.ds(j * D, D)
            return pltpu.make_async_copy(wm_hbm.at[:, cols], wmbuf.at[j], sem_wm.at[j])

        def q_copy(b):
            rows = pl.ds(b * TM, TM)
            return pltpu.make_async_copy(q_hbm.at[0, rows, :], qbuf.at[rows, :], sem_q.at[b])

        def w_copies(j):
            cols = pl.ds(j * FC, FC)
            return [
                pltpu.make_async_copy(w1_hbm.at[:, cols], w1buf.at[j], sem_w.at[0, j]),
                pltpu.make_async_copy(w3_hbm.at[:, cols], w3buf.at[j], sem_w.at[1, j]),
                pltpu.make_async_copy(w2_hbm.at[cols, :], w2buf.at[j], sem_w.at[2, j]),
            ]

        def o_copy(b):
            rows = pl.ds(pl.multiple_of(b * TM, TM), TM)
            return pltpu.make_async_copy(obuf.at[rows, :], o_hbm.at[0, rows, :], sem_o.at[b])

        def start(cs):
            for cp in cs:
                cp.start()

        def wait(cs):
            for cp in cs:
                cp.wait()

        s_copy(0).start()
        s_copy(1).start()
        start(conv_copies(0))

        sh = shift_ref[...].astype(F32)
        dd = d_ref[...].astype(F32).reshape(1, D)
        for t in range(NT):
            taps[t, 0:4, :] = sh[:, t * LANES:(t + 1) * LANES]
            taps[t, 4:5, :] = dd[:, t * LANES:(t + 1) * LANES]
            kbuf[t, 0:16, :] = jnp.zeros((16, LANES), BF)

        def as_rows(x):
            return pltpu.bitcast(x, F32).reshape(x.shape[0] // 16, 8, LANES)

        def from_rows(x):
            return pltpu.bitcast(x.reshape(x.shape[0] * 8, LANES), BF)

        for p in range(2):
            zb[pl.ds(F_OFF + 16 * p, 16)] = as_rows(fm_ref[p])
            for h in range(2):
                zb[pl.ds(G_OFF + 16 * p + 8 * h, 8)] = as_rows(gm_ref[p, :, h * LANES:(h + 1) * LANES])

        def transpose_taps(t, i):
            st = sbuf[t, :, pl.ds(pl.multiple_of(i * C, C), C)].T
            sw = pltpu.bitcast(st, U32)
            for p in range(2):
                zb[pl.ds(T_OFF + ((t % 2) * NCH + i) * 16 + 8 * p, 8)] = as_rows(_unpack(sw, p).astype(BF))

        def conv_step(i, tt, tf, ts, ti, order):
            env = {"F": [], "G": []}
            nf, ng = order.count("F"), order.count("G")
            pieces = [(h, f1, m) for h in range(2) for f1 in range(2) for m in range(3)]

            def short_conv():
                h0 = pl.multiple_of(i * (C // 2), C // 2)
                kw = kbuf.bitcast(U32)
                p0, p1, p2 = (kw[tf, pl.ds(h0 + 8 - n, C // 2), :] for n in range(3))
                ke, ko = _unpack(p0, 0), _unpack(p0, 1)
                ke1, ko1 = _unpack(p1, 0), _unpack(p1, 1)
                ko2 = _unpack(p2, 1)
                vw = vbuf.bitcast(U32)[tf, pl.ds(h0, C // 2), :]
                w0, w1, w2, w3 = (taps[tf, j:j + 1, :] for j in range(4))
                env["kv"] = [((w0 * ke + w1 * ko1 + w2 * ke1 + w3 * ko2) * _unpack(vw, 0)).astype(BF),
                             ((w0 * ko + w1 * ke + w2 * ko1 + w3 * ke1) * _unpack(vw, 1)).astype(BF)]
                env["kt"] = [from_rows(zb[pl.ds(T_OFF + ((tf % 2) * NCH + i) * 16 + 8 * p, 8)]) for p in range(2)]

            def load_f():
                j, m = len(env["F"]), 16 // nf
                env["F"].append([from_rows(zb[pl.ds(F_OFF + 16 * p + j * m, m)]) for p in range(2)])

            def load_g():
                j, m = len(env["G"]), 8 // ng
                env["G"].append([jnp.concatenate(
                    [from_rows(zb[pl.ds(G_OFF + 16 * p + 8 * h + j * m, m)]) for h in range(2)], axis=1)
                    for p in range(2)])

            def forward():
                fm = [jnp.concatenate([f[p] for f in env["F"]], axis=0) for p in range(2)]
                skip = jnp.where(i == 0, jnp.broadcast_to(taps[tf, 4:5, :], (8, LANES)), 0.0)
                for dst, x, dre in (((xs0, xs1)[tf % 2], env["kv"], None), ((ks0, ks1)[tf % 2], env["kt"], skip)):
                    e, o = _dot(fm[0], x[0]), _dot(fm[1], x[1])
                    for j in range(16):
                        er, ei = e[16 * j:16 * j + 8], e[16 * j + 8:16 * j + 16]
                        orr, oi = o[16 * j:16 * j + 8], o[16 * j + 8:16 * j + 16]
                        if dre is not None:
                            er = er + dre
                        dst[j, 0, 0, i] = er + orr
                        dst[j, 0, 1, i] = ei + oi
                        dst[j, 1, 0, i] = er - orr
                        dst[j, 1, 1, i] = ei - oi

            def product():
                xs, ks = (xs0, xs1)[ts % 2], (ks0, ks1)[ts % 2]
                half, f1, m = pieces.pop(0)
                j = i + 8 * half
                sub, add = ((jnp.subtract, jnp.add), (jnp.add, jnp.subtract))[half]

                def ld(ref, n):
                    return [ref[j, f1, n, c] for c in range(NCH)]
                cr, ci = ld(ks, 0), ld(ks, 1)
                if m == 0:
                    x = ld(xs, 0)
                    k = [cr[0]] + [sub(cr[n], ci[n - 1]) for n in range(1, NCH)]
                elif m == 1:
                    x = ld(xs, 1)
                    k = [ci[0]] + [add(ci[n], cr[n - 1]) for n in range(1, NCH)]
                else:
                    x = [u + w for u, w in zip(ld(xs, 0), ld(xs, 1))]
                    k = [cr[0] + ci[0]] + [add(cr[n] + ci[n], cr[n - 1] - ci[n - 1]) for n in range(1, NCH)]
                out = _causal_conv(x, k)
                for c in range(NCH):
                    zb[((ts % 2) * NCH + c) * 96 + j * 6 + f1 * 3 + m] = out[c]

            def combine():
                base = ((ti % 2) * NCH + i) * 96
                v0, v1 = [], []
                for j in range(16):
                    z = []
                    for f1 in range(2):
                        p, q, r = (zb[base + j * 6 + f1 * 3 + m] for m in range(3))
                        z.append((p - q, r - p - q))
                    v0.append(_pack(z[0][0] + z[1][0], z[0][1] + z[1][1]))
                    v1.append(_pack(z[0][0] - z[1][0], z[0][1] - z[1][1]))
                env["v"] = [pltpu.bitcast(jnp.concatenate(v, axis=0), BF) for v in (v0, v1)]

            def inverse():
                gm = [jnp.concatenate([g[p] for g in env["G"]], axis=0) for p in range(2)]
                ye, yo = _dot(gm[0], env["v"][0]), _dot(gm[1], env["v"][1])
                ybuf[ti, pl.ds(pl.multiple_of(i * C, C), C), :] = pltpu.bitcast(_pack(ye, yo), BF)

            ops = {"t": (tt, lambda: transpose_taps(tt, i)), "k": (tf, short_conv), "F": (tf, load_f),
                   "X": (tf, forward), "b": (ts, product), "c": (ti, combine), "G": (ti, load_g),
                   "Y": (ti, inverse)}
            for ch in order:
                tile, fn = ops[ch]
                if tile is not None:
                    fn()

        def stage(tt, tf, ts, ti):
            def step(i, carry):
                for u in range(UNROLL):
                    conv_step(i * UNROLL + u, tt, tf, ts, ti, ORDER)
                return carry
            lax.fori_loop(0, NCH // UNROLL, step, 0)

        cc = c_ref[...].astype(F32)
        sc = jnp.broadcast_to(cc * jax.nn.sigmoid(cc), (16, D)).astype(BF)

        def mod_part(j):
            wm_copy(j).wait()
            mod[j] = _dot(sc, wmbuf[j])[0:8]

        def tile(t):
            return t if 0 <= t < NT else None

        s_copy(0).wait()
        stage(0, None, None, None)
        for it in range(NT + 2):
            if it + 2 < NT:
                s_copy(it + 2).start()
            if it + 1 < NT:
                start(conv_copies(it + 1))
            if it == 3:
                for j in range(5):
                    wm_copy(j).start()
                q_copy(0).start()
            if it == 4:
                start(w_copies(0))
                q_copy(1).start()
            if it == 5:
                for j in range(1, NFC):
                    start(w_copies(j))
                wm_copy(5).start()
            if it == 6:
                for b in range(2, NB):
                    q_copy(b).start()
            if it + 1 < NT:
                s_copy(it + 1).wait()
            if it < NT:
                wait(conv_copies(it))
            if do_conv:
                stage(tile(it + 1), tile(it), tile(it - 1), tile(it - 2))
        if not do_conv:
            for t in range(NT):
                ybuf[t] = vbuf[t]
        for j in range(5):
            mod_part(j)

        def pre(b, x1buf, h2buf):
            rows = pl.ds(pl.multiple_of(b * TM, TM), TM)
            sa, ca, ga, sb, cb = (mod[j, 0:1, :] for j in range(5))
            x = qbuf[rows, :].astype(F32)
            y = jnp.concatenate([ybuf[t, rows, :] for t in range(NT)], axis=1).astype(F32)
            h = _layernorm(x) * (1 + ca) + sa
            x1 = x + ga * (h * y)
            x1buf[...] = x1
            h2buf[...] = (_layernorm(x1) * (1 + cb) + sb).astype(BF)

        def ffn(b, x1buf, h2buf, first=False):
            rows = pl.ds(pl.multiple_of(b * TM, TM), TM)
            h2 = h2buf[...]
            acc = None
            for j in range(NFC):
                if first:
                    wait(w_copies(j))
                g = _dot(h2, w1buf[j])
                u = _dot(h2, w3buf[j])
                a = (g * jax.nn.sigmoid(g) * u).astype(BF)
                p = _dot(a, w2buf[j])
                acc = p if acc is None else acc + p
            if first:
                mod_part(5)
            obuf[rows, :] = (x1buf[...] + mod[5, 0:1, :] * acc).astype(BF)
            o_copy(b).start()

        q_copy(0).wait()
        pre(0, x1a, h2a)
        q_copy(1).wait()
        pre(1, x1b, h2b)
        ffn(0, x1a, h2a, True)
        for b in range(2, NB):
            q_copy(b).wait()

        def blk(b, carry):
            b = 2 * b + 1
            pre(b + 1, x1a, h2a)
            ffn(b, x1b, h2b)
            pre(b + 2, x1b, h2b)
            ffn(b + 1, x1a, h2a)
            return carry
        lax.fori_loop(0, NB // 2 - 1, blk, 0)
        ffn(NB - 1, x1b, h2b)
        for b in range(NB):
            o_copy(b).wait()

    fm, gm = _dft_consts()
    any_spec = pl.BlockSpec(memory_space=pl.ANY)
    vmem_spec = pl.BlockSpec(memory_space=pltpu.VMEM)

    @jax.jit
    def kernel(A_q, A_k, A_v, A_shift_k, A_ssm_k, A_ssm_D, B_x, B_w1, B_w3, B_w2, c, w_mod):
        del B_x
        return pl.pallas_call(
            body,
            out_shape=jax.ShapeDtypeStruct((1, S, D), BF),
            in_specs=[any_spec, any_spec, any_spec, vmem_spec, any_spec, vmem_spec,
                      any_spec, any_spec, any_spec, vmem_spec, any_spec, vmem_spec, vmem_spec],
            out_specs=any_spec,
            scratch_shapes=[
                pltpu.VMEM((NT, S + 16, LANES), BF),
                pltpu.VMEM((NT, S, LANES), BF),
                pltpu.VMEM((NT, LANES, S), BF),
                pltpu.VMEM((S, D), BF),
                pltpu.VMEM((NFC, D, FC), BF),
                pltpu.VMEM((NFC, D, FC), BF),
                pltpu.VMEM((NFC, FC, D), BF),
                pltpu.VMEM((6, D, D), BF),
                pltpu.VMEM((NT, S, LANES), BF),
                pltpu.VMEM((S, D), BF),
                pltpu.VMEM((16, 2, 2, NCH, 8, LANES), F32),
                pltpu.VMEM((16, 2, 2, NCH, 8, LANES), F32),
                pltpu.VMEM((16, 2, 2, NCH, 8, LANES), F32),
                pltpu.VMEM((16, 2, 2, NCH, 8, LANES), F32),
                pltpu.VMEM((Z_ROWS, 8, LANES), F32),
                pltpu.VMEM((NT, 8, LANES), F32),
                pltpu.VMEM((6, 8, D), F32),
                pltpu.VMEM((TM, D), F32),
                pltpu.VMEM((TM, D), F32),
                pltpu.VMEM((TM, D), BF),
                pltpu.VMEM((TM, D), BF),
                pltpu.SemaphoreType.DMA((3, NT)),
                pltpu.SemaphoreType.DMA((6,)),
                pltpu.SemaphoreType.DMA((NB,)),
                pltpu.SemaphoreType.DMA((3, NFC)),
                pltpu.SemaphoreType.DMA((NB,)),
            ],
            compiler_params=pltpu.CompilerParams(vmem_limit_bytes=100 * 2**20, flags=flags),
        )(A_q, A_k, A_v, A_shift_k.T, A_ssm_k, A_ssm_D, B_w1, B_w3, B_w2, c, w_mod,
          jnp.asarray(fm), jnp.asarray(gm))
    return kernel


pallas_adaLN_cond__ssm_conv_h3__glu_gated_swiglu__prompt_kernel = make()
```

```python
import contextlib
import numpy as np
import jax
import jax.numpy as jnp
from jax import lax
import jax.experimental.pallas as pl
import jax.experimental.pallas.tpu as pltpu

S, D, F = 2048, 640, 1536
LANES = 128
NT = D // LANES
C = 256
NB = S // C
NPOS = 16
BF, F32, U32 = jnp.bfloat16, jnp.float32, jnp.uint32

Z_CHUNK = NPOS * 2 * 3
T_OFF = NT * NB * Z_CHUNK
F_OFF = T_OFF + NB * 16
Z_ROWS = F_OFF + 33


def _dft_consts():
    L = 2 * C
    u = np.concatenate([np.arange(0, 64, 2), np.arange(1, 64, 2)])
    f0 = np.concatenate([u, 127 - u])
    fm = np.zeros((2, 256, 128), np.float32)
    for p in range(2):
        th = 2 * np.pi * np.outer(f0 + 0.5, 2 * np.arange(128) + p) / L
        fm[p] = np.stack([np.cos(th).reshape(16, 8, 128), -np.sin(th).reshape(16, 8, 128)], axis=1).reshape(256, 128)
    gm = np.zeros((4, 64, 128), np.float32)
    for p in range(4):
        th = 2 * np.pi * np.outer(4 * np.arange(64) + p, u + 0.5) / L
        gm[p, :, 0::2] = (2 / L) * np.cos(th)
        gm[p, :, 1::2] = -(2 / L) * np.sin(th)

    def row_pairs(m):
        h = m.astype(BF).view(np.uint16).astype(np.uint32)
        return h[:, 0::2] | (h[:, 1::2] << 16)
    return row_pairs(fm), row_pairs(gm)


def _unpack(w, i):
    return pltpu.unpack_elementwise(w, index=i, packed_dtype=BF, unpacked_dtype=F32)


def _pack(lo, hi):
    return pltpu.pack_elementwise([lo, hi], packed_dtype=BF)


def _dot(a, b):
    return jnp.dot(a, b, preferred_element_type=F32)


def _causal_conv(x, k):
    out = []
    for i in range(len(x)):
        acc = x[i] * k[0]
        for j in range(1, i + 1):
            acc = acc + x[i - j] * k[j]
        out.append(acc)
    return out


def _layernorm(x):
    m = jnp.mean(x, axis=-1, keepdims=True)
    xc = x - m
    v = jnp.mean(xc * xc, axis=-1, keepdims=True)
    return xc * lax.rsqrt(v + 1e-5)


def _silu(x):
    h = 0.5 * x
    return h + h * jnp.tanh(h)


PLAN = [
    ("g0", [""] * 4), "I0", "I1",
    ("u0", [""] * 4), "I2", "I3",
    ("d0", [""] * 5), "I4",
    ("g1", ["", "P0", "P1", "P2"]),
    ("u1", ["P3", "P4", "P5", "P6"]),
    ("d1", ["P7", "", "P8", "", "P9"]),
    ("g2", ["P10", "P11", "P12", "P13"]),
    ("u2", ["P14", "P15", "", ""]),
    ("d2", [""] * 5),
]


def make(FC=512, order="kFbFbFbFbFbFbFtbFbbbbbX", plan=PLAN, npre=16,
         flags=None, scopes=False, issue_at=(0, 1, 3, 4, 5, 6, 7, 8, 10, 11, 12, 13, 15, 16, 18)):
    NFC = F // FC
    CPC = FC // LANES
    scope = (lambda n: jax.named_scope('S_' + n)) if scopes else (lambda n: contextlib.nullcontext())

    def body(q_hbm, k_hbm, v_hbm, shift_ref, s_hbm, d_ref, w1_hbm, w3_hbm, w2_hbm, c_ref, wm_hbm,
             fm_ref, gm_ref, o_hbm,
             kbuf, vbuf, sbuf, qbuf, w1buf, w3buf, w2buf, wmbuf, ybuf, obuf,
             xs0, xs1, ks0, ks1, zb, taps, mod, x1buf, h2buf,
             sem_in, sem_wm, sem_q, sem_w, sem_o):

        def block_rows(b):
            return pl.ds(pl.multiple_of(b * C, C), C)

        def lanes(t):
            return pl.ds(t * LANES, LANES)

        def s_copy(t):
            return [pltpu.make_async_copy(s_hbm.at[lanes(t), :], sbuf.at[t], sem_in.at[0, t])]

        def k_copy(t):
            return [pltpu.make_async_copy(k_hbm.at[0, :, lanes(t)], kbuf.at[t, pl.ds(16, S), :], sem_in.at[1, t])]

        def v_copy(t):
            return [pltpu.make_async_copy(v_hbm.at[0, :, lanes(t)], vbuf.at[t], sem_in.at[2, t])]

        def wm_copy(j):
            return [pltpu.make_async_copy(wm_hbm.at[:, pl.ds(j * D, D)], wmbuf.at[j], sem_wm.at[j])]

        def q_copy(b):
            return [pltpu.make_async_copy(q_hbm.at[0, block_rows(b), :], qbuf.at[block_rows(b), :], sem_q.at[b])]

        def w1_copy(j):
            return [pltpu.make_async_copy(w1_hbm.at[:, pl.ds(j * FC, FC)], w1buf.at[j], sem_w.at[0, j])]

        def w3_copy(j):
            return [pltpu.make_async_copy(w3_hbm.at[:, pl.ds(j * FC, FC)], w3buf.at[j], sem_w.at[1, j])]

        def w2_copy(j):
            return [pltpu.make_async_copy(w2_hbm.at[pl.ds(j * FC, FC), :], w2buf.at[j], sem_w.at[2, j])]

        def o_copy(b):
            return [pltpu.make_async_copy(obuf.at[block_rows(b), :], o_hbm.at[0, block_rows(b), :], sem_o.at[b])]

        def start(copies):
            for cp in copies:
                cp.start()

        def wait(copies):
            for cp in copies:
                cp.wait()

        def as_regs(x):
            return pltpu.bitcast(x, F32).reshape(x.shape[0] // 16, 8, LANES)

        def from_regs(x):
            return pltpu.bitcast(x.reshape(x.shape[0] * 8, LANES), BF)

        def transpose_taps(n):
            cols = pl.ds(pl.multiple_of(n % NB * C, C), C)
            sw = pltpu.bitcast(sbuf[n // NB, :, cols].T, U32)
            for p in range(2):
                zb[pl.ds(T_OFF + n % NB * 16 + 8 * p, 8)] = as_regs(_unpack(sw, p).astype(BF))

        def conv_step(i, tf, ts):
            fparts, env = [], {}
            pieces = [(h, f1, m) for h in range(2) for f1 in range(2) for m in range(3)]

            def short_conv():
                h0 = pl.multiple_of(i * (C // 2), C // 2)
                kw = kbuf.bitcast(U32)
                p0, p1, p2 = (kw[tf, pl.ds(h0 + 8 - n, C // 2), :] for n in range(3))
                ke, ko = _unpack(p0, 0), _unpack(p0, 1)
                ke1, ko1 = _unpack(p1, 0), _unpack(p1, 1)
                ko2 = _unpack(p2, 1)
                vw = vbuf.bitcast(U32)[tf, pl.ds(h0, C // 2), :]
                w0, w1, w2, w3 = (taps[tf, j:j + 1, :] for j in range(4))
                env["kv"] = [((w0 * ke + w1 * ko1 + w2 * ke1 + w3 * ko2) * _unpack(vw, 0)).astype(BF),
                             ((w0 * ko + w1 * ke + w2 * ko1 + w3 * ke1) * _unpack(vw, 1)).astype(BF)]
                env["kt"] = [from_regs(zb[pl.ds(T_OFF + i * 16 + 8 * p, 8)]) for p in range(2)]

            def load_dft():
                n = 16 // order.count("F")
                fparts.append([from_regs(zb[pl.ds(F_OFF + 16 * p + len(fparts) * n, n)]) for p in range(2)])

            def forward():
                fm = [jnp.concatenate([f[p] for f in fparts], axis=0) for p in range(2)]
                skip = jnp.where(i == 0, jnp.broadcast_to(taps[tf, 4:5, :], (8, LANES)), 0.0)
                for dst, x, lag0 in (((xs0, xs1)[tf % 2], env["kv"], None), ((ks0, ks1)[tf % 2], env["kt"], skip)):
                    e, o = _dot(fm[0], x[0]), _dot(fm[1], x[1])
                    for j in range(NPOS):
                        re, im = slice(16 * j, 16 * j + 8), slice(16 * j + 8, 16 * j + 16)
                        er = e[re] if lag0 is None else e[re] + lag0
                        dst[j, 0, 0, i], dst[j, 0, 1, i] = er + o[re], e[im] + o[im]
                        dst[j, 1, 0, i], dst[j, 1, 1, i] = er - o[re], e[im] - o[im]

            def product():
                xs, ks = (xs0, xs1)[ts % 2], (ks0, ks1)[ts % 2]
                odd, f1, m = pieces.pop(0)
                j = i + 4 if odd else (i + 12) % NPOS
                sub, add = (jnp.add, jnp.subtract) if odd else (jnp.subtract, jnp.add)

                def ld(ref, n):
                    return [ref[j, f1, n, c] for c in range(NB)]
                kr, ki = ld(ks, 0), ld(ks, 1)
                if m == 0:
                    x = ld(xs, 0)
                    k = [kr[0]] + [sub(kr[n], ki[n - 1]) for n in range(1, NB)]
                elif m == 1:
                    x = ld(xs, 1)
                    k = [ki[0]] + [add(ki[n], kr[n - 1]) for n in range(1, NB)]
                else:
                    x = [u + w for u, w in zip(ld(xs, 0), ld(xs, 1))]
                    k = [kr[0] + ki[0]] + [add(kr[n] + ki[n], kr[n - 1] - ki[n - 1]) for n in range(1, NB)]
                for c, z in enumerate(_causal_conv(x, k)):
                    zb[(ts * NB + c) * Z_CHUNK + j * 6 + f1 * 3 + m] = z

            def taps_ahead():
                transpose_taps(jnp.minimum(tf * NB + i + NB // 2, NT * NB - 1))

            ops = {"t": (tf, taps_ahead), "k": (tf, short_conv), "F": (tf, load_dft),
                   "X": (tf, forward), "b": (ts, product)}
            for ch in order:
                tile, fn = ops[ch]
                if tile is not None:
                    fn()

        def stage(t, events):
            def step(i, carry):
                for at, fn in events.items():
                    pl.when(i == at)(fn)
                for u in range(2):
                    conv_step(2 * i + u, t, t - 1 if t else None)
                return carry
            lax.fori_loop(0, NB // 2, step, 0)

        def inverse(b, t):
            base = (t * NB + b) * Z_CHUNK

            def position(j):
                z = []
                for f1 in range(2):
                    p, q, r = (zb[base + j * 6 + f1 * 3 + m] for m in range(3))
                    z.append((p - q, r - p - q))
                return (z[0][0] + z[1][0], z[0][1] + z[1][1]), (z[0][0] - z[1][0], z[0][1] - z[1][1])

            w = [[], [], [], []]
            for j in range(NPOS // 2):
                (r0, i0), (r1, i1) = position(j)
                (x0, y0), (x1, y1) = position(j + NPOS // 2)
                for p, (re, im) in enumerate(((r0 + x0, i0 - y0), (r1 - y1, i1 - x1),
                                              (r0 - x0, i0 + y0), (r1 + y1, i1 + x1))):
                    w[p].append(_pack(re, im))
            y = [_dot(pltpu.bitcast(gm_ref[p], BF), pltpu.bitcast(jnp.concatenate(w[p], axis=0), BF))
                 for p in range(4)]
            ybuf[t, pl.ds(0, C // 4, stride=2), :] = _pack(y[0], y[1])
            ybuf[t, pl.ds(1, C // 4, stride=2), :] = _pack(y[2], y[3])

        def pre(b, r, n):
            sa, ca, ga, sb, cb = (mod[j, 0:1, :] for j in range(5))
            x = qbuf[pl.ds(pl.multiple_of(b * C + r, n), n), :].astype(F32)
            y = jnp.concatenate([pltpu.bitcast(ybuf[t, r // 2:(r + n) // 2, :], BF) for t in range(NT)], axis=1)
            h = _layernorm(x) * (1 + ca) + sa
            x1 = x + ga * (h * y.astype(F32))
            x1buf[b % 2, r:r + n, :] = x1
            h2 = pltpu.bitcast((_layernorm(x1) * (1 + cb) + sb).astype(BF), U32)
            for t in range(NT):
                h2buf[b % 2, t, r // 2:(r + n) // 2, :] = h2[:, t * LANES:(t + 1) * LANES]
            return h2[n // 2 - 8:n // 2, 0:LANES]

        cc = c_ref[...].astype(F32)
        sc = jnp.broadcast_to(_silu(cc), (16, D)).astype(BF)

        def mod_part(j):
            mod[j] = _dot(sc, wmbuf[j])[0:8]

        def mlp(b, zero, last=False, before=None):
            def matmul(x, wbuf, j, fill):
                cols = []
                for n, items in enumerate(fill):
                    cols.append(wbuf[j, :, n * LANES:(n + 1) * LANES])
                    for item in ([] if last else items.split()):
                        done = pre(b + 1, int(item[1:]) * (C // npre), C // npre)
                        wbuf[NFC + zero, 0:16, 0:LANES] = pltpu.bitcast(done, BF)
                out = _dot(x, jnp.concatenate(cols, axis=1))
                if not last:
                    for buf in (w1buf, w3buf, w2buf):
                        buf[NFC + zero, 16:32, 0:LANES] = pltpu.bitcast(out[0:8, 0:LANES], BF)
                    zb[Z_ROWS - 1 + zero] = out[0:8, 0:LANES]
                return out

            h2 = jnp.concatenate([pltpu.bitcast(h2buf[b % 2, t], BF) for t in range(NT)], axis=1)
            g, a, acc = {}, {}, None
            for o in plan:
                if isinstance(o, str):
                    if not last:
                        inverse(b + 1, int(o[1:]))
                    continue
                if before and o[0] in before:
                    before[o[0]]()
                kind, j = o[0][0], int(o[0][1:])
                if kind == "g":
                    g[j] = matmul(h2, w1buf, j, o[1])
                elif kind == "u":
                    a[j] = (_silu(g[j]) * matmul(h2, w3buf, j, o[1])).astype(BF)
                else:
                    p = matmul(a[j], w2buf, j, o[1])
                    acc = p if acc is None else acc + p
            if before:
                before["out"]()
            obuf[block_rows(b), :] = (x1buf[b % 2] + mod[5, 0:1, :] * acc).astype(BF)
            start(o_copy(b))

        start(s_copy(0) + k_copy(0))
        sh = shift_ref[...].astype(F32)
        dd = d_ref[...].astype(F32).reshape(1, D)
        for t in range(NT):
            taps[t, 0:4, :] = sh[:, t * LANES:(t + 1) * LANES]
            taps[t, 4:5, :] = dd[:, t * LANES:(t + 1) * LANES]
        kbuf[:, 0:16, :] = jnp.zeros((NT, 16, LANES), BF)
        for p in range(2):
            zb[pl.ds(F_OFF + 16 * p, 16)] = pltpu.bitcast(fm_ref[p], F32).reshape(16, 8, LANES)
        with scope("tr0"):
            wait(s_copy(0))
            start(v_copy(0))
            for n in range(NB // 2):
                transpose_taps(n)
            wait(k_copy(0))
            start(s_copy(1))
        queue = [lambda t=t, copy=copy: copy(t) for t in range(1, NT) for copy in (s_copy, k_copy, v_copy)][1:]
        queue += [lambda j=j: wm_copy(j) for j in range(4)]
        issue = dict(zip(issue_at, queue))
        for t in range(NT):
            def event(i, t=t):
                def fn():
                    if t * NB // 2 + i in issue:
                        start(issue[t * NB // 2 + i]())
                    if i == NB // 4 and t + 1 < NT:
                        wait(s_copy(t + 1))
                return fn
            with scope("w%d" % t):
                wait((k_copy(t) if t else []) + v_copy(t))
            with scope("st%d" % t):
                stage(t, {i: event(i) for i in range(NB // 2)})
        with scope("st5"):
            start(wm_copy(4))
            for i in range(NB):
                if i == 2:
                    wait(wm_copy(0) + wm_copy(1) + wm_copy(2))
                    start(q_copy(0) + w1_copy(0))
                if i == 6:
                    wait(wm_copy(3) + wm_copy(4))
                    start(w3_copy(0))
                if i in (2, 3, 4, 6, 7):
                    mod_part((2, 3, 4, 6, 7).index(i))
                if i < NT - 1:
                    inverse(0, i)
                conv_step(i, None, NT - 1)
        with scope("pre0"):
            inverse(0, NT - 1)
            wait(q_copy(0))
            start(w2_copy(0) + q_copy(1))
            pre(0, 0, C)

        def arrive(copies, then):
            def fn():
                wait(copies())
                start(then())
            return fn

        def gate_out():
            wait(wm_copy(5))
            start([cp for b in range(2, NB) for cp in q_copy(b)])
            mod_part(5)

        def first(b, carry):
            mlp(b, pl.program_id(0), before={
                "g0": arrive(lambda: w1_copy(0) + w3_copy(0), lambda: w1_copy(1) + w3_copy(1)),
                "d0": arrive(lambda: w2_copy(0) + q_copy(1) + w1_copy(1), lambda: w2_copy(1) + w1_copy(2)),
                "u1": arrive(lambda: w3_copy(1) + w2_copy(1), lambda: w3_copy(2) + w2_copy(2)),
                "g2": arrive(lambda: w1_copy(2) + w3_copy(2), lambda: wm_copy(5)),
                "d2": arrive(lambda: w2_copy(2), lambda: []),
                "out": gate_out})
            return carry

        def middle(b, carry):
            wait(q_copy(b + 1))
            mlp(b, b // NB)
            return carry

        with scope("mlp0"):
            first(0, 0)
        with scope("loop"):
            lax.fori_loop(1, NB - 1, middle, 0)
        with scope("last"):
            mlp(NB - 1, 0, last=True)
        with scope("wout"):
            for b in range(NB):
                wait(o_copy(b))

    fm, gm = _dft_consts()
    any_spec = pl.BlockSpec(memory_space=pl.ANY)
    vmem_spec = pl.BlockSpec(memory_space=pltpu.VMEM)
    spectrum = pltpu.VMEM((NPOS, 2, 2, NB, 8, LANES), F32)

    @jax.jit
    def kernel(A_q, A_k, A_v, A_shift_k, A_ssm_k, A_ssm_D, B_x, B_w1, B_w3, B_w2, c, w_mod):
        del B_x
        return pl.pallas_call(
            body,
            grid=(1,),
            out_shape=jax.ShapeDtypeStruct((1, S, D), BF),
            in_specs=[any_spec, any_spec, any_spec, vmem_spec, any_spec, vmem_spec,
                      any_spec, any_spec, any_spec, vmem_spec, any_spec, vmem_spec, vmem_spec],
            out_specs=any_spec,
            scratch_shapes=[
                pltpu.VMEM((NT, S + 16, LANES), BF),
                pltpu.VMEM((NT, S, LANES), BF),
                pltpu.VMEM((NT, LANES, S), BF),
                pltpu.VMEM((S, D), BF),
                pltpu.VMEM((NFC + 1, D, FC), BF),
                pltpu.VMEM((NFC + 1, D, FC), BF),
                pltpu.VMEM((NFC + 1, FC, D), BF),
                pltpu.VMEM((6, D, D), BF),
                pltpu.VMEM((NT, C // 2, LANES), U32),
                pltpu.VMEM((S, D), BF),
                spectrum, spectrum, spectrum, spectrum,
                pltpu.VMEM((Z_ROWS, 8, LANES), F32),
                pltpu.VMEM((NT, 8, LANES), F32),
                pltpu.VMEM((6, 8, D), F32),
                pltpu.VMEM((2, C, D), F32),
                pltpu.VMEM((2, NT, C // 2, LANES), U32),
                pltpu.SemaphoreType.DMA((3, NT)),
                pltpu.SemaphoreType.DMA((6,)),
                pltpu.SemaphoreType.DMA((NB,)),
                pltpu.SemaphoreType.DMA((3, NFC)),
                pltpu.SemaphoreType.DMA((NB,)),
            ],
            compiler_params=pltpu.CompilerParams(vmem_limit_bytes=100 * 2**20, flags=flags),
        )(A_q, A_k, A_v, A_shift_k.T, A_ssm_k, A_ssm_D, B_w1, B_w3, B_w2, c, w_mod,
          jnp.asarray(fm), jnp.asarray(gm))
    return kernel


pallas_adaLN_cond__ssm_conv_h3__glu_gated_swiglu__prompt_kernel = make()
```

```python
import contextlib
import numpy as np
import jax
import jax.numpy as jnp
from jax import lax
import jax.experimental.pallas as pl
import jax.experimental.pallas.tpu as pltpu

S, D, F = 2048, 640, 1536
LANES = 128
NT = D // LANES
C = 256
NB = S // C
NPOS = 16
BF, F32, U32 = jnp.bfloat16, jnp.float32, jnp.uint32

Z_CHUNK = NPOS * 2 * 3
T_OFF = NT * NB * Z_CHUNK
F_OFF = T_OFF + NB * 16
Z_ROWS = F_OFF + 33


def _dft_consts():
    L = 2 * C
    u = np.concatenate([np.arange(0, 64, 2), np.arange(1, 64, 2)])
    f0 = np.concatenate([u, 127 - u])
    fm = np.zeros((2, 256, 128), np.float32)
    for p in range(2):
        th = 2 * np.pi * np.outer(f0 + 0.5, 2 * np.arange(128) + p) / L
        fm[p] = np.stack([np.cos(th).reshape(16, 8, 128), -np.sin(th).reshape(16, 8, 128)], axis=1).reshape(256, 128)
    gm = np.zeros((4, 64, 128), np.float32)
    for p in range(4):
        th = 2 * np.pi * np.outer(4 * np.arange(64) + p, u + 0.5) / L
        gm[p, :, 0::2] = (2 / L) * np.cos(th)
        gm[p, :, 1::2] = -(2 / L) * np.sin(th)

    def row_pairs(m):
        h = m.astype(BF).view(np.uint16).astype(np.uint32)
        return h[:, 0::2] | (h[:, 1::2] << 16)
    return row_pairs(fm).view(np.float32).reshape(32, 8, 128), row_pairs(gm)


def _unpack(w, i):
    return pltpu.unpack_elementwise(w, index=i, packed_dtype=BF, unpacked_dtype=F32)


def _pack(lo, hi):
    return pltpu.pack_elementwise([lo, hi], packed_dtype=BF)


def _dot(a, b):
    return jnp.dot(a, b, preferred_element_type=F32)


def _causal_conv(x, k):
    out = []
    for i in range(len(x)):
        acc = x[i] * k[0]
        for j in range(1, i + 1):
            acc = acc + x[i - j] * k[j]
        out.append(acc)
    return out


def _layernorm(x):
    m = jnp.mean(x, axis=-1, keepdims=True)
    xc = x - m
    v = jnp.mean(xc * xc, axis=-1, keepdims=True)
    return xc * lax.rsqrt(v + 1e-5)


def _silu(x):
    h = 0.5 * x
    return h + h * jnp.tanh(h)


PLAN = [
    ("g0", [""] * 4), "I0", "I1",
    ("u0", [""] * 4), "I2", "I3",
    ("d0", [""] * 5), "I4",
    ("g1", ["", "P0", "P1", "P2"]),
    ("u1", ["P3", "P4", "P5", "P6"]),
    ("d1", ["P7", "", "P8", "", "P9"]),
    ("g2", ["P10", "P11", "P12", "P13"]),
    ("u2", ["P14", "P15", "", ""]),
    ("d2", [""] * 5),
]


def _plan(text):
    plan = []
    for part in text.split("|"):
        name, *fill = part.split(",")
        plan.append(name.strip() if not fill else (name.strip(), fill))
    return plan


def make(FC=512, order=("kFbFbFbFbFbFbFtbFbbbbbX",) * 2, plan=PLAN, npre=16,
         flags=None, scopes=False, only_conv=False, unroll=1, issue_at=(0, 1, 3, 4, 5, 6, 7, 8, 10, 11, 12, 13, 15, 16, 18)):
    NFC = F // FC
    plan = _plan(plan) if isinstance(plan, str) else plan
    CPC = FC // LANES
    scope = (lambda n: jax.named_scope('S_' + n)) if scopes else (lambda n: contextlib.nullcontext())

    def body(q_hbm, k_hbm, v_hbm, shift_hbm, s_hbm, d_hbm, w1_hbm, w3_hbm, w2_hbm, c_hbm, wm_hbm,
             fm_hbm, gm_hbm, o_hbm, shift_ref, d_ref, c_ref, gm_ref,
             kbuf, vbuf, sbuf, qbuf, w1buf, w3buf, w2buf, wmbuf, ybuf, obuf,
             xs0, xs1, ks0, ks1, zb, taps, mod, x1buf, h2buf,
             sem_in, sem_wm, sem_q, sem_w, sem_o, sem_small):

        def block_rows(b):
            return pl.ds(pl.multiple_of(b * C, C), C)

        def lanes(t):
            return pl.ds(t * LANES, LANES)

        def s_copy(t):
            return [pltpu.make_async_copy(s_hbm.at[lanes(t), :], sbuf.at[t], sem_in.at[0, t])]

        def k_copy(t):
            return [pltpu.make_async_copy(k_hbm.at[0, :, lanes(t)], kbuf.at[t, pl.ds(16, S), :], sem_in.at[1, t])]

        def v_copy(t):
            return [pltpu.make_async_copy(v_hbm.at[0, :, lanes(t)], vbuf.at[t], sem_in.at[2, t])]

        def wm_copy(j):
            return [pltpu.make_async_copy(wm_hbm.at[:, pl.ds(j * D, D)], wmbuf.at[j], sem_wm.at[j])]

        def q_copy(b):
            return [pltpu.make_async_copy(q_hbm.at[0, block_rows(b), :], qbuf.at[block_rows(b), :], sem_q.at[b])]

        def w1_copy(j):
            return [pltpu.make_async_copy(w1_hbm.at[:, pl.ds(j * FC, FC)], w1buf.at[j], sem_w.at[0, j])]

        def w3_copy(j):
            return [pltpu.make_async_copy(w3_hbm.at[:, pl.ds(j * FC, FC)], w3buf.at[j], sem_w.at[1, j])]

        def w2_copy(j):
            return [pltpu.make_async_copy(w2_hbm.at[pl.ds(j * FC, FC), :], w2buf.at[j], sem_w.at[2, j])]

        def o_copy(b):
            return [pltpu.make_async_copy(obuf.at[block_rows(b), :], o_hbm.at[0, block_rows(b), :], sem_o.at[b])]

        def start(copies):
            for cp in copies:
                cp.start()

        def wait(copies):
            for cp in copies:
                cp.wait()

        def as_regs(x):
            return pltpu.bitcast(x, F32).reshape(x.shape[0] // 16, 8, LANES)

        def from_regs(x):
            return pltpu.bitcast(x.reshape(x.shape[0] * 8, LANES), BF)

        def transpose_taps(n):
            cols = pl.ds(pl.multiple_of(n % NB * C, C), C)
            sw = pltpu.bitcast(sbuf[n // NB, :, cols].T, U32)
            for p in range(2):
                zb[pl.ds(T_OFF + n % NB * 16 + 8 * p, 8)] = as_regs(_unpack(sw, p).astype(BF))

        def conv_step(i, tf, ts, order="b" * 12):
            fparts, env = [], {}
            pieces = [(h, f1, m) for h in range(2) for f1 in range(2) for m in range(3)]

            def short_conv():
                h0 = pl.multiple_of(i * (C // 2), C // 2)
                kw = kbuf.bitcast(U32)
                p0, p1, p2 = (kw[tf, pl.ds(h0 + 8 - n, C // 2), :] for n in range(3))
                ke, ko = _unpack(p0, 0), _unpack(p0, 1)
                ke1, ko1 = _unpack(p1, 0), _unpack(p1, 1)
                ko2 = _unpack(p2, 1)
                vw = vbuf.bitcast(U32)[tf, pl.ds(h0, C // 2), :]
                w0, w1, w2, w3 = (taps[tf, j:j + 1, :] for j in range(4))
                env["kv"] = [((w0 * ke + w1 * ko1 + w2 * ke1 + w3 * ko2) * _unpack(vw, 0)).astype(BF),
                             ((w0 * ko + w1 * ke + w2 * ko1 + w3 * ke1) * _unpack(vw, 1)).astype(BF)]
                env["kt"] = [from_regs(zb[pl.ds(T_OFF + i * 16 + 8 * p, 8)]) for p in range(2)]

            def load_dft():
                n = 16 // order.count("F")
                fparts.append([from_regs(zb[pl.ds(F_OFF + 16 * p + len(fparts) * n, n)]) for p in range(2)])

            def forward():
                fm = [jnp.concatenate([f[p] for f in fparts], axis=0) for p in range(2)]
                skip = jnp.where(i == 0, jnp.broadcast_to(taps[tf, 4:5, :], (8, LANES)), 0.0)
                for dst, x, lag0 in (((xs0, xs1)[tf % 2], env["kv"], None), ((ks0, ks1)[tf % 2], env["kt"], skip)):
                    e, o = _dot(fm[0], x[0]), _dot(fm[1], x[1])
                    for j in range(NPOS):
                        re, im = slice(16 * j, 16 * j + 8), slice(16 * j + 8, 16 * j + 16)
                        er = e[re] if lag0 is None else e[re] + lag0
                        dst[j, 0, 0, i], dst[j, 0, 1, i] = er + o[re], e[im] + o[im]
                        dst[j, 1, 0, i], dst[j, 1, 1, i] = er - o[re], e[im] - o[im]

            def product():
                xs, ks = (xs0, xs1)[ts % 2], (ks0, ks1)[ts % 2]
                odd, f1, m = pieces.pop(0)
                j = i + 4 if odd else (i + 12) % NPOS
                sub, add = (jnp.add, jnp.subtract) if odd else (jnp.subtract, jnp.add)

                def ld(ref, n):
                    return [ref[j, f1, n, c] for c in range(NB)]
                kr, ki = ld(ks, 0), ld(ks, 1)
                if m == 0:
                    x = ld(xs, 0)
                    k = [kr[0]] + [sub(kr[n], ki[n - 1]) for n in range(1, NB)]
                elif m == 1:
                    x = ld(xs, 1)
                    k = [ki[0]] + [add(ki[n], kr[n - 1]) for n in range(1, NB)]
                else:
                    x = [u + w for u, w in zip(ld(xs, 0), ld(xs, 1))]
                    k = [kr[0] + ki[0]] + [add(kr[n] + ki[n], kr[n - 1] - ki[n - 1]) for n in range(1, NB)]
                for c, z in enumerate(_causal_conv(x, k)):
                    zb[(ts * NB + c) * Z_CHUNK + j * 6 + f1 * 3 + m] = z

            def taps_ahead():
                transpose_taps(jnp.minimum(tf * NB + i + NB // 2, NT * NB - 1))

            ops = {"t": (tf, taps_ahead), "k": (tf, short_conv), "F": (tf, load_dft),
                   "X": (tf, forward), "b": (ts, product)}
            for ch in order:
                tile, fn = ops[ch]
                if tile is not None:
                    fn()

        def stage(t, events):
            def step(i, carry):
                for at, fn in events.items():
                    pl.when(i == at)(fn)
                for u in range(2):
                    conv_step(2 * i + u, t, t - 1 if t else None, order[u])
                return carry
            lax.fori_loop(0, NB // 2, step, 0)

        def inverse(b, t):
            base = (t * NB + b) * Z_CHUNK

            def position(j):
                z = []
                for f1 in range(2):
                    p, q, r = (zb[base + j * 6 + f1 * 3 + m] for m in range(3))
                    z.append((p - q, r - p - q))
                return (z[0][0] + z[1][0], z[0][1] + z[1][1]), (z[0][0] - z[1][0], z[0][1] - z[1][1])

            w = [[], [], [], []]
            for j in range(NPOS // 2):
                (r0, i0), (r1, i1) = position(j)
                (x0, y0), (x1, y1) = position(j + NPOS // 2)
                for p, (re, im) in enumerate(((r0 + x0, i0 - y0), (r1 - y1, i1 - x1),
                                              (r0 - x0, i0 + y0), (r1 + y1, i1 + x1))):
                    w[p].append(_pack(re, im))
            y = [_dot(pltpu.bitcast(gm_ref[p], BF), pltpu.bitcast(jnp.concatenate(w[p], axis=0), BF))
                 for p in range(4)]
            ybuf[t, pl.ds(0, C // 4, stride=2), :] = _pack(y[0], y[1])
            ybuf[t, pl.ds(1, C // 4, stride=2), :] = _pack(y[2], y[3])

        def pre(b, r, n):
            sa, ca, ga, sb, cb = (mod[j, 0:1, :] for j in range(5))
            x = qbuf[pl.ds(pl.multiple_of(b * C + r, n), n), :].astype(F32)
            y = jnp.concatenate([pltpu.bitcast(ybuf[t, r // 2:(r + n) // 2, :], BF) for t in range(NT)], axis=1)
            h = _layernorm(x) * (1 + ca) + sa
            x1 = x + ga * (h * y.astype(F32))
            x1buf[b % 2, r:r + n, :] = x1
            h2 = pltpu.bitcast((_layernorm(x1) * (1 + cb) + sb).astype(BF), U32)
            for t in range(NT):
                h2buf[b % 2, t, r // 2:(r + n) // 2, :] = h2[:, t * LANES:(t + 1) * LANES]
            return h2[n // 2 - 8:n // 2, 0:LANES]

        def mod_part(j):
            sc = jnp.broadcast_to(_silu(c_ref[...].astype(F32)), (16, D)).astype(BF)
            mod[j] = _dot(sc, wmbuf[j])[0:8]

        def mlp(b, zero, last=False, before=None):
            def matmul(x, wbuf, j, fill):
                cols = []
                for n, items in enumerate(fill):
                    cols.append(wbuf[j, :, n * LANES:(n + 1) * LANES])
                    for item in ([] if last else items.split()):
                        done = pre(b + 1, int(item[1:]) * (C // npre), C // npre)
                        wbuf[NFC + zero, 0:16, 0:LANES] = pltpu.bitcast(done, BF)
                out = _dot(x, jnp.concatenate(cols, axis=1))
                if not last:
                    for buf in (w1buf, w3buf, w2buf):
                        buf[NFC + zero, 16:32, 0:LANES] = pltpu.bitcast(out[0:8, 0:LANES], BF)
                    zb[Z_ROWS - 1 + zero] = out[0:8, 0:LANES]
                return out

            h2 = jnp.concatenate([pltpu.bitcast(h2buf[b % 2, t], BF) for t in range(NT)], axis=1)
            g, a, acc = {}, {}, None
            for o in plan:
                if isinstance(o, str):
                    if not last:
                        inverse(b + 1, int(o[1:]))
                    continue
                if before and o[0] in before:
                    with scope(o[0]):
                        before[o[0]]()
                kind, j = o[0][0], int(o[0][1:])
                if kind == "g":
                    g[j] = matmul(h2, w1buf, j, o[1])
                elif kind == "u":
                    a[j] = (_silu(g[j]) * matmul(h2, w3buf, j, o[1])).astype(BF)
                else:
                    p = matmul(a[j], w2buf, j, o[1])
                    acc = p if acc is None else acc + p
            obuf[block_rows(b), :] = (x1buf[b % 2] + mod[5, 0:1, :] * acc).astype(BF)
            start(o_copy(b))

        small = [pltpu.make_async_copy(src, dst, sem_small) for src, dst in (
            (shift_hbm, shift_ref), (d_hbm, d_ref), (c_hbm, c_ref), (gm_hbm, gm_ref),
            (fm_hbm, zb.at[pl.ds(F_OFF, 32)]))]
        start(s_copy(0) + small + k_copy(0))
        kbuf[:, 0:16, :] = jnp.zeros((NT, 16, LANES), BF)
        with scope("tr0"):
            wait(s_copy(0))
            start(v_copy(0))
            for n in range(NB // 2):
                transpose_taps(n)
            wait(small)
            sh = shift_ref[...].astype(F32)
            dd = d_ref[...].astype(F32).reshape(1, D)
            for t in range(NT):
                taps[t, 0:4, :] = sh[:, t * LANES:(t + 1) * LANES]
                taps[t, 4:5, :] = dd[:, t * LANES:(t + 1) * LANES]
            wait(k_copy(0))
            start(s_copy(1))
        queue = [lambda t=t, copy=copy: copy(t) for t in range(1, NT) for copy in (s_copy, k_copy, v_copy)][1:]
        queue += [lambda j=j: wm_copy(j) for j in range(4)]
        issue = dict(zip(issue_at, queue))
        for t in range(NT):
            def event(i, t=t):
                def fn():
                    if t * NB // 2 + i in issue:
                        start(issue[t * NB // 2 + i]())
                    if i == NB // 4 and t + 1 < NT:
                        wait(s_copy(t + 1))
                return fn
            with scope("w%d" % t):
                wait((k_copy(t) if t else []) + v_copy(t))
            with scope("st%d" % t):
                stage(t, {i: event(i) for i in range(NB // 2)})
        with scope("st5"):
            start(wm_copy(4))
            for i in range(NB):
                if i == 2:
                    wait(wm_copy(0) + wm_copy(1) + wm_copy(2))
                    start(q_copy(0) + w1_copy(0))
                if i == 6:
                    wait(wm_copy(3) + wm_copy(4))
                    start(w3_copy(0))
                if i in (2, 3, 4, 6, 7):
                    mod_part((2, 3, 4, 6, 7).index(i))
                if i < NT - 1:
                    inverse(0, i)
                conv_step(i, None, NT - 1)
        with scope("pre0"):
            inverse(0, NT - 1)
            wait(q_copy(0))
            start(w2_copy(0) + q_copy(1))
            pre(0, 0, C)

        def arrive(copies, then):
            def fn():
                wait(copies())
                start(then())
            return fn

        def gate_out():
            wait(w2_copy(2) + wm_copy(5))
            start([cp for b in range(2, NB) for cp in q_copy(b)])
            mod_part(5)

        def first(b, carry):
            mlp(b, pl.program_id(0), before={
                "g0": arrive(lambda: w1_copy(0) + w3_copy(0), lambda: w1_copy(1) + w3_copy(1)),
                "d0": arrive(lambda: w2_copy(0) + q_copy(1) + w1_copy(1), lambda: w2_copy(1) + w1_copy(2)),
                "u1": arrive(lambda: w3_copy(1) + w2_copy(1), lambda: w3_copy(2) + w2_copy(2) + wm_copy(5)),
                "g2": arrive(lambda: w1_copy(2) + w3_copy(2), lambda: []),
                "d2": gate_out})
            return carry

        def middle(i, carry):
            for u in range(unroll):
                wait(q_copy(unroll * i + u + 2))
            for u in range(unroll):
                mlp(unroll * i + u + 1, i // NB)
            return carry

        if only_conv:
            obuf[0:C, :] = x1buf[0].astype(BF)
            start(o_copy(0))
            wait(o_copy(0))
            return
        with scope("mlp0"):
            first(0, 0)
        with scope("loop"):
            lax.fori_loop(0, (NB - 2) // unroll, middle, 0)
        with scope("last"):
            mlp(NB - 1, 0, last=True)
        with scope("wout"):
            for b in range(NB):
                wait(o_copy(b))

    fm, gm = _dft_consts()
    any_spec = pl.BlockSpec(memory_space=pl.ANY)
    spectrum = pltpu.VMEM((NPOS, 2, 2, NB, 8, LANES), F32)

    @jax.jit
    def kernel(A_q, A_k, A_v, A_shift_k, A_ssm_k, A_ssm_D, B_x, B_w1, B_w3, B_w2, c, w_mod):
        del B_x
        return pl.pallas_call(
            body,
            grid=(1,),
            out_shape=jax.ShapeDtypeStruct((1, S, D), BF),
            in_specs=[any_spec] * 13,
            out_specs=any_spec,
            scratch_shapes=[
                pltpu.VMEM((4, D), BF),
                pltpu.VMEM((D,), BF),
                pltpu.VMEM((1, D), BF),
                pltpu.VMEM((4, 32, LANES), U32),
                pltpu.VMEM((NT, S + 16, LANES), BF),
                pltpu.VMEM((NT, S, LANES), BF),
                pltpu.VMEM((NT, LANES, S), BF),
                pltpu.VMEM((S, D), BF),
                pltpu.VMEM((NFC + 1, D, FC), BF),
                pltpu.VMEM((NFC + 1, D, FC), BF),
                pltpu.VMEM((NFC + 1, FC, D), BF),
                pltpu.VMEM((6, D, D), BF),
                pltpu.VMEM((NT, C // 2, LANES), U32),
                pltpu.VMEM((S, D), BF),
                spectrum, spectrum, spectrum, spectrum,
                pltpu.VMEM((Z_ROWS, 8, LANES), F32),
                pltpu.VMEM((NT, 8, LANES), F32),
                pltpu.VMEM((6, 8, D), F32),
                pltpu.VMEM((2, C, D), F32),
                pltpu.VMEM((2, NT, C // 2, LANES), U32),
                pltpu.SemaphoreType.DMA((3, NT)),
                pltpu.SemaphoreType.DMA((6,)),
                pltpu.SemaphoreType.DMA((NB,)),
                pltpu.SemaphoreType.DMA((3, NFC)),
                pltpu.SemaphoreType.DMA((NB,)),
                pltpu.SemaphoreType.DMA(()),
            ],
            compiler_params=pltpu.CompilerParams(vmem_limit_bytes=100 * 2**20, flags=flags),
        )(A_q, A_k, A_v, A_shift_k.T, A_ssm_k, A_ssm_D, B_w1, B_w3, B_w2, c, w_mod,
          jnp.asarray(fm), jnp.asarray(gm))
    return kernel


pallas_adaLN_cond__ssm_conv_h3__glu_gated_swiglu__prompt_kernel = make()
```

```python
import contextlib
import numpy as np
import jax
import jax.numpy as jnp
from jax import lax
import jax.experimental.pallas as pl
import jax.experimental.pallas.tpu as pltpu

S, D, F = 2048, 640, 1536
LANES = 128
NT = D // LANES
C = 256
NB = S // C
NPOS = 16
BF, F32, U32 = jnp.bfloat16, jnp.float32, jnp.uint32

Z_CHUNK = NPOS * 2 * 3
T_OFF = NT * NB * Z_CHUNK
F_OFF = T_OFF + NB * 16
Z_ROWS = F_OFF + 33


def _dft_consts():
    L = 2 * C
    u = np.concatenate([np.arange(0, 64, 2), np.arange(1, 64, 2)])
    f0 = np.concatenate([u, 127 - u])
    fm = np.zeros((2, 256, 128), np.float32)
    for p in range(2):
        th = 2 * np.pi * np.outer(f0 + 0.5, 2 * np.arange(128) + p) / L
        fm[p] = np.stack([np.cos(th).reshape(16, 8, 128), -np.sin(th).reshape(16, 8, 128)], axis=1).reshape(256, 128)
    gm = np.zeros((4, 64, 128), np.float32)
    for p in range(4):
        th = 2 * np.pi * np.outer(4 * np.arange(64) + p, u + 0.5) / L
        gm[p, :, 0::2] = (2 / L) * np.cos(th)
        gm[p, :, 1::2] = -(2 / L) * np.sin(th)

    def row_pairs(m):
        h = m.astype(BF).view(np.uint16).astype(np.uint32)
        return h[:, 0::2] | (h[:, 1::2] << 16)
    return row_pairs(fm).view(np.float32).reshape(32, 8, 128), row_pairs(gm)


def _unpack(w, i):
    return pltpu.unpack_elementwise(w, index=i, packed_dtype=BF, unpacked_dtype=F32)


def _pack(lo, hi):
    return pltpu.pack_elementwise([lo, hi], packed_dtype=BF)


def _dot(a, b):
    return jnp.dot(a, b, preferred_element_type=F32)


def _causal_conv(x, k):
    out = []
    for i in range(len(x)):
        acc = x[i] * k[0]
        for j in range(1, i + 1):
            acc = acc + x[i - j] * k[j]
        out.append(acc)
    return out


def _layernorm(x):
    m = jnp.mean(x, axis=-1, keepdims=True)
    xc = x - m
    v = jnp.mean(xc * xc, axis=-1, keepdims=True)
    return xc * lax.rsqrt(v + 1e-5)


def _silu(x):
    h = 0.5 * x
    return h + h * jnp.tanh(h)


PLAN = "g0,,,,|I0|I1|u0,,,,|I2|I3|d0,,,,,|I4|g1,,P0,,P1|u1,P2,P3,P4,P5|d1,P6,,P7,,P8|g2,P9,P10,P11,P12|u2,P13,P14,P15,|d2,,,,,"


def _plan(text):
    plan = []
    for part in text.split("|"):
        name, *fill = part.split(",")
        plan.append(name.strip() if not fill else (name.strip(), fill))
    return plan


def make(FC=512, order=("kFbbFbFbbFbFbbFbFtbbFbX", "kFbbFbFbFbbFtbFbFbFbbbX"), plan=PLAN, npre=16,
         flags=None, scopes=False, only_conv=False, unroll=1, issue_at=(0, 1, 2, 4, 5, 6, 7, 8, 10, 11, 12, 13, 14, 16, 18)):
    NFC = F // FC
    plan = _plan(plan) if isinstance(plan, str) else plan
    CPC = FC // LANES
    scope = (lambda n: jax.named_scope('S_' + n)) if scopes else (lambda n: contextlib.nullcontext())

    def body(q_hbm, k_hbm, v_hbm, shift_hbm, s_hbm, d_hbm, w1_hbm, w3_hbm, w2_hbm, c_hbm, wm_hbm,
             fm_hbm, gm_hbm, o_hbm, shift_ref, d_ref, c_ref, gm_ref,
             kbuf, vbuf, sbuf, qbuf, w1buf, w3buf, w2buf, wmbuf, ybuf, obuf,
             xs0, xs1, ks0, ks1, zb, carry, taps, mod, x1buf, h2buf,
             sem_in, sem_wm, sem_q, sem_w, sem_o, sem_small):

        def block_rows(b):
            return pl.ds(pl.multiple_of(b * C, C), C)

        def lanes(t):
            return pl.ds(t * LANES, LANES)

        def s_copy(t):
            return [pltpu.make_async_copy(s_hbm.at[lanes(t), :], sbuf.at[t], sem_in.at[0, t])]

        def k_copy(t):
            return [pltpu.make_async_copy(k_hbm.at[0, :, lanes(t)], kbuf.at[t, pl.ds(16, S), :], sem_in.at[1, t])]

        def v_copy(t):
            return [pltpu.make_async_copy(v_hbm.at[0, :, lanes(t)], vbuf.at[t], sem_in.at[2, t])]

        def wm_copy(j):
            return [pltpu.make_async_copy(wm_hbm.at[:, pl.ds(j * D, D)], wmbuf.at[j], sem_wm.at[j])]

        def q_copy(b):
            return [pltpu.make_async_copy(q_hbm.at[0, block_rows(b), :], qbuf.at[block_rows(b), :], sem_q.at[b])]

        def w1_copy(j):
            return [pltpu.make_async_copy(w1_hbm.at[:, pl.ds(j * FC, FC)], w1buf.at[j], sem_w.at[0, j])]

        def w3_copy(j):
            return [pltpu.make_async_copy(w3_hbm.at[:, pl.ds(j * FC, FC)], w3buf.at[j], sem_w.at[1, j])]

        def w2_copy(j):
            return [pltpu.make_async_copy(w2_hbm.at[pl.ds(j * FC, FC), :], w2buf.at[j], sem_w.at[2, j])]

        def o_copy(b):
            return [pltpu.make_async_copy(obuf.at[block_rows(b), :], o_hbm.at[0, block_rows(b), :], sem_o.at[b])]

        def start(copies):
            for cp in copies:
                cp.start()

        def wait(copies):
            for cp in copies:
                cp.wait()

        def as_regs(x):
            return pltpu.bitcast(x, F32).reshape(x.shape[0] // 16, 8, LANES)

        def from_regs(x):
            return pltpu.bitcast(x.reshape(x.shape[0] * 8, LANES), BF)

        def transpose_taps(n):
            cols = pl.ds(pl.multiple_of(n % NB * C, C), C)
            sw = pltpu.bitcast(sbuf[n // NB, :, cols].T, U32)
            for p in range(2):
                zb[pl.ds(T_OFF + n % NB * 16 + 8 * p, 8)] = as_regs(_unpack(sw, p).astype(BF))

        def conv_step(i, tf, ts, order="b" * 12):
            fparts, env = [], {}
            pieces = [(h, f1, m) for h in range(2) for f1 in range(2) for m in range(3)]

            def short_conv():
                h0 = pl.multiple_of(i * (C // 2), C // 2)
                kw = kbuf.bitcast(U32)
                p0, p1, p2 = (kw[tf, pl.ds(h0 + 8 - n, C // 2), :] for n in range(3))
                ke, ko = _unpack(p0, 0), _unpack(p0, 1)
                ke1, ko1 = _unpack(p1, 0), _unpack(p1, 1)
                ko2 = _unpack(p2, 1)
                vw = vbuf.bitcast(U32)[tf, pl.ds(h0, C // 2), :]
                w0, w1, w2, w3 = (taps[tf, j:j + 1, :] for j in range(4))
                env["kv"] = [((w0 * ke + w1 * ko1 + w2 * ke1 + w3 * ko2) * _unpack(vw, 0)).astype(BF),
                             ((w0 * ko + w1 * ke + w2 * ko1 + w3 * ke1) * _unpack(vw, 1)).astype(BF)]
                env["kt"] = [from_regs(zb[pl.ds(T_OFF + i * 16 + 8 * p, 8)]) for p in range(2)]

            def load_dft():
                n = 16 // order.count("F")
                fparts.append([from_regs(zb[pl.ds(F_OFF + 16 * p + len(fparts) * n, n)]) for p in range(2)])

            def forward():
                fm = [jnp.concatenate([f[p] for f in fparts], axis=0) for p in range(2)]
                skip = jnp.where(i == 0, jnp.broadcast_to(taps[tf, 4:5, :], (8, LANES)), 0.0)
                for dst, x, lag0 in (((xs0, xs1)[tf % 2], env["kv"], None), ((ks0, ks1)[tf % 2], env["kt"], skip)):
                    e, o = _dot(fm[0], x[0]), _dot(fm[1], x[1])
                    for j in range(NPOS):
                        re, im = slice(16 * j, 16 * j + 8), slice(16 * j + 8, 16 * j + 16)
                        er = e[re] if lag0 is None else e[re] + lag0
                        dst[j, 0, 0, i], dst[j, 0, 1, i] = er + o[re], e[im] + o[im]
                        dst[j, 1, 0, i], dst[j, 1, 1, i] = er - o[re], e[im] - o[im]

            def product():
                xs, ks = (xs0, xs1)[ts % 2], (ks0, ks1)[ts % 2]
                half, f1, m = pieces.pop(0)
                j = i + half * (NPOS // 2)

                def operand(ref):
                    if m < 2:
                        return [ref[j, f1, m, c] for c in range(NB)]
                    return [ref[j, f1, 0, c] + ref[j, f1, 1, c] for c in range(NB)]
                x, k = operand(xs), operand(ks)
                for c, z in enumerate(_causal_conv(x, k)):
                    zb[(ts * NB + c) * Z_CHUNK + j * 6 + f1 * 3 + m] = z

            def taps_ahead():
                transpose_taps(jnp.minimum(tf * NB + i + NB // 2, NT * NB - 1))

            ops = {"t": (tf, taps_ahead), "k": (tf, short_conv), "F": (tf, load_dft),
                   "X": (tf, forward), "b": (ts, product)}
            for ch in order:
                tile, fn = ops[ch]
                if tile is not None:
                    fn()

        def stage(t, events):
            def step(i, _):
                for at, fn in events.items():
                    pl.when(i == at)(fn)
                for u in range(2):
                    conv_step(2 * i + u, t, t - 1 if t else None, order[u])
                return 0
            lax.fori_loop(0, NB // 2, step, 0)

        def inverse(b, t):
            base = (t * NB + b) * Z_CHUNK

            def position(j):
                z = []
                for f1 in range(2):
                    p, q, r = (zb[base + j * 6 + f1 * 3 + m] for m in range(3))
                    z.append((p - q, r - p - q))
                out = []
                for p, op in enumerate((jnp.add, jnp.subtract)):
                    re, im = op(z[0][0], z[1][0]), op(z[0][1], z[1][1])
                    if isinstance(b, int) and b == 0:
                        out.append((re, im))
                    elif NPOS // 4 <= j < 3 * NPOS // 4:
                        out.append((re + carry[t, j, p, 1], im - carry[t, j, p, 0]))
                    else:
                        out.append((re - carry[t, j, p, 1], im + carry[t, j, p, 0]))
                    carry[t, j, p, 0], carry[t, j, p, 1] = re, im
                return out

            w = [[], [], [], []]
            for j in range(NPOS // 2):
                (r0, i0), (r1, i1) = position(j)
                (x0, y0), (x1, y1) = position(j + NPOS // 2)
                for p, (re, im) in enumerate(((r0 + x0, i0 - y0), (r1 - y1, i1 - x1),
                                              (r0 - x0, i0 + y0), (r1 + y1, i1 + x1))):
                    w[p].append(_pack(re, im))
            y = [_dot(pltpu.bitcast(gm_ref[p], BF), pltpu.bitcast(jnp.concatenate(w[p], axis=0), BF))
                 for p in range(4)]
            ybuf[t, pl.ds(0, C // 4, stride=2), :] = _pack(y[0], y[1])
            ybuf[t, pl.ds(1, C // 4, stride=2), :] = _pack(y[2], y[3])

        def pre(b, r, n):
            sa, ca1, ga, sb, cb1 = (jnp.concatenate([mod[j]] * (n // 8), axis=0) for j in range(5))
            x = qbuf[pl.ds(pl.multiple_of(b * C + r, n), n), :].astype(F32)
            y = jnp.concatenate([pltpu.bitcast(ybuf[t, r // 2:(r + n) // 2, :], BF) for t in range(NT)], axis=1)
            h = _layernorm(x) * ca1 + sa
            x1 = x + ga * (h * y.astype(F32))
            x1buf[b % 2, r:r + n, :] = x1
            h2 = pltpu.bitcast((_layernorm(x1) * cb1 + sb).astype(BF), U32)
            for t in range(NT):
                h2buf[b % 2, t, r // 2:(r + n) // 2, :] = h2[:, t * LANES:(t + 1) * LANES]
            return h2[n // 2 - 8:n // 2, 0:LANES]

        def mod_part(j):
            sc = jnp.broadcast_to(_silu(c_ref[...].astype(F32)), (16, D)).astype(BF)
            part = _dot(sc, wmbuf[j])[0:8]
            mod[j] = 1 + part if j in (1, 4) else part

        def mlp(b, zero, last=False, before=None):
            def matmul(x, wbuf, j, fill):
                cols = []
                for n, items in enumerate(fill):
                    cols.append(wbuf[j, :, n * LANES:(n + 1) * LANES])
                    for item in ([] if last else items.split()):
                        done = pre(b + 1, int(item[1:]) * (C // npre), C // npre)
                        wbuf[NFC + zero, 0:16, 0:LANES] = pltpu.bitcast(done, BF)
                out = _dot(x, jnp.concatenate(cols, axis=1))
                if not last:
                    for buf in (w1buf, w3buf, w2buf):
                        buf[NFC + zero, 16:32, 0:LANES] = pltpu.bitcast(out[0:8, 0:LANES], BF)
                    zb[Z_ROWS - 1 + zero] = out[0:8, 0:LANES]
                return out

            h2 = jnp.concatenate([pltpu.bitcast(h2buf[b % 2, t], BF) for t in range(NT)], axis=1)
            g, a, acc = {}, {}, None
            for o in plan:
                if isinstance(o, str):
                    if not last:
                        inverse(b + 1, int(o[1:]))
                    continue
                if before and o[0] in before:
                    with scope(o[0]):
                        before[o[0]]()
                kind, j = o[0][0], int(o[0][1:])
                if kind == "g":
                    g[j] = matmul(h2, w1buf, j, o[1])
                elif kind == "u":
                    a[j] = (_silu(g[j]) * matmul(h2, w3buf, j, o[1])).astype(BF)
                else:
                    p = matmul(a[j], w2buf, j, o[1])
                    acc = p if acc is None else acc + p
            gb = jnp.concatenate([mod[5]] * (C // 8), axis=0)
            obuf[block_rows(b), :] = (x1buf[b % 2] + gb * acc).astype(BF)
            start(o_copy(b))

        small = [pltpu.make_async_copy(src, dst, sem_small) for src, dst in (
            (shift_hbm, shift_ref), (d_hbm, d_ref), (c_hbm, c_ref), (gm_hbm, gm_ref),
            (fm_hbm, zb.at[pl.ds(F_OFF, 32)]))]
        start(s_copy(0) + small + k_copy(0))
        kbuf[:, 0:16, :] = jnp.zeros((NT, 16, LANES), BF)
        with scope("tr0"):
            wait(s_copy(0))
            start(v_copy(0))
            for n in range(NB // 2):
                transpose_taps(n)
            wait(small)
            sh = shift_ref[...].astype(F32)
            dd = d_ref[...].astype(F32).reshape(1, D)
            for t in range(NT):
                taps[t, 0:4, :] = sh[:, t * LANES:(t + 1) * LANES]
                taps[t, 4:5, :] = dd[:, t * LANES:(t + 1) * LANES]
            wait(k_copy(0))
            start(s_copy(1))
        queue = [lambda t=t, copy=copy: copy(t) for t in range(1, NT) for copy in (s_copy, k_copy, v_copy)][1:]
        queue += [lambda j=j: wm_copy(j) for j in range(4)]
        issue = dict(zip(issue_at, queue))
        for t in range(NT):
            def event(i, t=t):
                def fn():
                    if t * NB // 2 + i in issue:
                        start(issue[t * NB // 2 + i]())
                    if i == NB // 4 and t + 1 < NT:
                        wait(s_copy(t + 1))
                return fn
            with scope("w%d" % t):
                wait((k_copy(t) if t else []) + v_copy(t))
            with scope("st%d" % t):
                stage(t, {i: event(i) for i in range(NB // 2)})
        with scope("st5"):
            start(wm_copy(4))
            for i in range(NB):
                if i == 2:
                    wait(wm_copy(0) + wm_copy(1) + wm_copy(2))
                    start(q_copy(0) + w1_copy(0))
                if i == 6:
                    wait(wm_copy(3) + wm_copy(4))
                    start(w3_copy(0))
                if i in (2, 3, 4, 6, 7):
                    mod_part((2, 3, 4, 6, 7).index(i))
                if i < NT - 1:
                    inverse(0, i)
                conv_step(i, None, NT - 1)
        with scope("pre0"):
            inverse(0, NT - 1)
            wait(q_copy(0))
            start(w2_copy(0) + q_copy(1))
            pre(0, 0, C)

        def arrive(copies, then):
            def fn():
                wait(copies())
                start(then())
            return fn

        def gate_out():
            wait(w2_copy(2) + wm_copy(5))
            start([cp for b in range(2, NB) for cp in q_copy(b)])
            mod_part(5)

        def first(b, _):
            mlp(b, pl.program_id(0), before={
                "g0": arrive(lambda: w1_copy(0) + w3_copy(0), lambda: w1_copy(1) + w3_copy(1)),
                "d0": arrive(lambda: w2_copy(0) + q_copy(1) + w1_copy(1), lambda: w2_copy(1) + w1_copy(2)),
                "u1": arrive(lambda: w3_copy(1) + w2_copy(1), lambda: w3_copy(2) + w2_copy(2) + wm_copy(5)),
                "g2": arrive(lambda: w1_copy(2) + w3_copy(2), lambda: []),
                "d2": gate_out})
            return 0

        def middle(i, _):
            for u in range(unroll):
                wait(q_copy(unroll * i + u + 2))
            for u in range(unroll):
                mlp(unroll * i + u + 1, i // NB)
            return 0

        if only_conv:
            obuf[0:C, :] = x1buf[0].astype(BF)
            start(o_copy(0))
            wait(o_copy(0))
            return
        with scope("mlp0"):
            first(0, 0)
        with scope("loop"):
            lax.fori_loop(0, (NB - 2) // unroll, middle, 0)
        with scope("last"):
            mlp(NB - 1, 0, last=True)
        with scope("wout"):
            for b in range(NB):
                wait(o_copy(b))

    fm, gm = _dft_consts()
    any_spec = pl.BlockSpec(memory_space=pl.ANY)
    spectrum = pltpu.VMEM((NPOS, 2, 2, NB, 8, LANES), F32)

    @jax.jit
    def kernel(A_q, A_k, A_v, A_shift_k, A_ssm_k, A_ssm_D, B_x, B_w1, B_w3, B_w2, c, w_mod):
        del B_x
        return pl.pallas_call(
            body,
            grid=(1,),
            out_shape=jax.ShapeDtypeStruct((1, S, D), BF),
            in_specs=[any_spec] * 13,
            out_specs=any_spec,
            scratch_shapes=[
                pltpu.VMEM((4, D), BF),
                pltpu.VMEM((D,), BF),
                pltpu.VMEM((1, D), BF),
                pltpu.VMEM((4, 32, LANES), U32),
                pltpu.VMEM((NT, S + 16, LANES), BF),
                pltpu.VMEM((NT, S, LANES), BF),
                pltpu.VMEM((NT, LANES, S), BF),
                pltpu.VMEM((S, D), BF),
                pltpu.VMEM((NFC + 1, D, FC), BF),
                pltpu.VMEM((NFC + 1, D, FC), BF),
                pltpu.VMEM((NFC + 1, FC, D), BF),
                pltpu.VMEM((6, D, D), BF),
                pltpu.VMEM((NT, C // 2, LANES), U32),
                pltpu.VMEM((S, D), BF),
                spectrum, spectrum, spectrum, spectrum,
                pltpu.VMEM((Z_ROWS, 8, LANES), F32),
                pltpu.VMEM((NT, NPOS, 2, 2, 8, LANES), F32),
                pltpu.VMEM((NT, 8, LANES), F32),
                pltpu.VMEM((6, 8, D), F32),
                pltpu.VMEM((2, C, D), F32),
                pltpu.VMEM((2, NT, C // 2, LANES), U32),
                pltpu.SemaphoreType.DMA((3, NT)),
                pltpu.SemaphoreType.DMA((6,)),
                pltpu.SemaphoreType.DMA((NB,)),
                pltpu.SemaphoreType.DMA((3, NFC)),
                pltpu.SemaphoreType.DMA((NB,)),
                pltpu.SemaphoreType.DMA(()),
            ],
            compiler_params=pltpu.CompilerParams(vmem_limit_bytes=100 * 2**20, flags=flags),
        )(A_q, A_k, A_v, A_shift_k.T, A_ssm_k, A_ssm_D, B_w1, B_w3, B_w2, c, w_mod,
          jnp.asarray(fm), jnp.asarray(gm))
    return kernel


pallas_adaLN_cond__ssm_conv_h3__glu_gated_swiglu__prompt_kernel = make()
```

```python
import numpy as np
import jax
import jax.numpy as jnp
from jax import lax
import jax.experimental.pallas as pl
import jax.experimental.pallas.tpu as pltpu

S, D, F = 2048, 640, 1536
LANES = 128
NT = D // LANES
C = 256
NB = S // C
NPOS = 16
BF, F32, U32 = jnp.bfloat16, jnp.float32, jnp.uint32

Z_CHUNK = NPOS * 2 * 3
T_OFF = NT * NB * Z_CHUNK
F_OFF = T_OFF + NB * 16
Z_ROWS = F_OFF + 33


def _dft_consts():
    L = 2 * C
    u = np.concatenate([np.arange(0, 64, 2), np.arange(1, 64, 2)])
    f0 = np.concatenate([u, 127 - u])
    fm = np.zeros((2, 256, 128), np.float32)
    for p in range(2):
        th = 2 * np.pi * np.outer(f0 + 0.5, 2 * np.arange(128) + p) / L
        fm[p] = np.stack([np.cos(th).reshape(16, 8, 128), -np.sin(th).reshape(16, 8, 128)], axis=1).reshape(256, 128)
    gm = np.zeros((4, 64, 128), np.float32)
    for p in range(4):
        th = 2 * np.pi * np.outer(4 * np.arange(64) + p, u + 0.5) / L
        gm[p, :, 0::2] = (2 / L) * np.cos(th)
        gm[p, :, 1::2] = -(2 / L) * np.sin(th)

    def row_pairs(m):
        h = m.astype(BF).view(np.uint16).astype(np.uint32)
        return h[:, 0::2] | (h[:, 1::2] << 16)
    return row_pairs(fm).view(np.float32).reshape(32, 8, 128), row_pairs(gm)


def _unpack(w, i):
    return pltpu.unpack_elementwise(w, index=i, packed_dtype=BF, unpacked_dtype=F32)


def _pack(lo, hi):
    return pltpu.pack_elementwise([lo, hi], packed_dtype=BF)


def _dot(a, b):
    return jnp.dot(a, b, preferred_element_type=F32)


def _causal_conv(x, k):
    out = []
    for i in range(len(x)):
        acc = x[i] * k[0]
        for j in range(1, i + 1):
            acc = acc + x[i - j] * k[j]
        out.append(acc)
    return out


def _layernorm(x):
    m = jnp.mean(x, axis=-1, keepdims=True)
    xc = x - m
    v = jnp.mean(xc * xc, axis=-1, keepdims=True)
    return xc * lax.rsqrt(v + 1e-5)


def _silu(x):
    h = 0.5 * x
    return h + h * jnp.tanh(h)


FC = 512
NFC = F // FC
NPRE = 16

STEP_ORDER = ("kFbbFbFbbFbFbbFbFtbbFbX", "kFbbFbFbFbbFtbFbFbFbbbX")
BLOCK_ORDER = (
    ("g", 0, ("", "", "", "")), ("I", 0), ("I", 1),
    ("u", 0, ("", "", "", "")), ("I", 2), ("I", 3),
    ("d", 0, ("", "", "", "", "")), ("I", 4),
    ("g", 1, ("", "0", "", "1")),
    ("u", 1, ("2", "3", "4", "5")),
    ("d", 1, ("6", "", "7", "", "8")),
    ("g", 2, ("9", "10", "11", "12")),
    ("u", 2, ("13", "14", "15", "")),
    ("d", 2, ("", "", "", "", "")),
)
ISSUE_AT = (0, 1, 2, 4, 5, 6, 7, 8, 10, 11, 12, 13, 14, 16, 18)


def _body(q_hbm, k_hbm, v_hbm, shift_hbm, s_hbm, d_hbm, w1_hbm, w3_hbm, w2_hbm, c_hbm, wm_hbm,
         fm_hbm, gm_hbm, o_hbm, shift_ref, d_ref, c_ref, gm_ref,
         kbuf, vbuf, sbuf, qbuf, w1buf, w3buf, w2buf, wmbuf, wgbuf, ybuf, obuf,
         xs0, xs1, ks0, ks1, zb, carry, taps, mod, gate, x1buf, h2buf,
         sem_in, sem_wm, sem_q, sem_w, sem_o, sem_small):

    def block_rows(b):
        return pl.ds(pl.multiple_of(b * C, C), C)

    def lanes(t):
        return pl.ds(t * LANES, LANES)

    def s_copy(t):
        return [pltpu.make_async_copy(s_hbm.at[lanes(t), :], sbuf.at[t], sem_in.at[0, t])]

    def k_copy(t):
        return [pltpu.make_async_copy(k_hbm.at[0, :, lanes(t)], kbuf.at[t, pl.ds(16, S), :], sem_in.at[1, t])]

    def v_copy(t):
        return [pltpu.make_async_copy(v_hbm.at[0, :, lanes(t)], vbuf.at[t], sem_in.at[2, t])]

    def wm_copy(j):
        return [pltpu.make_async_copy(wm_hbm.at[lanes(j), pl.ds(0, 5 * D)], wmbuf.at[j], sem_wm.at[j])]

    def gate_copy():
        return [pltpu.make_async_copy(wm_hbm.at[:, pl.ds(5 * D, D)], wgbuf, sem_wm.at[NT])]

    def q_copy(b):
        return [pltpu.make_async_copy(q_hbm.at[0, block_rows(b), :], qbuf.at[block_rows(b), :], sem_q.at[b])]

    def w1_copy(j):
        return [pltpu.make_async_copy(w1_hbm.at[:, pl.ds(j * FC, FC)], w1buf.at[j], sem_w.at[0, j])]

    def w3_copy(j):
        return [pltpu.make_async_copy(w3_hbm.at[:, pl.ds(j * FC, FC)], w3buf.at[j], sem_w.at[1, j])]

    def w2_copy(j):
        return [pltpu.make_async_copy(w2_hbm.at[pl.ds(j * FC, FC), :], w2buf.at[j], sem_w.at[2, j])]

    def o_copy(b):
        return [pltpu.make_async_copy(obuf.at[block_rows(b), :], o_hbm.at[0, block_rows(b), :], sem_o.at[b])]

    def tail_copy(t):
        rows = block_rows(NB - 1)
        return pltpu.make_async_copy(obuf.at[rows, lanes(t)], o_hbm.at[0, rows, lanes(t)], sem_o.at[NB - 1])

    def start(copies):
        for cp in copies:
            cp.start()

    def wait(copies):
        for cp in copies:
            cp.wait()

    def as_regs(x):
        return pltpu.bitcast(x, F32).reshape(x.shape[0] // 16, 8, LANES)

    def from_regs(x):
        return pltpu.bitcast(x.reshape(x.shape[0] * 8, LANES), BF)

    def transpose_taps(n):
        cols = pl.ds(pl.multiple_of(n % NB * C, C), C)
        sw = pltpu.bitcast(sbuf[n // NB, :, cols].T, U32)
        for p in range(2):
            zb[pl.ds(T_OFF + n % NB * 16 + 8 * p, 8)] = as_regs(_unpack(sw, p).astype(BF))

    def conv_step(i, tf, ts, order="b" * 12):
        fparts, env = [], {}
        pieces = [(h, f1, m) for h in range(2) for f1 in range(2) for m in range(3)]

        def short_conv():
            h0 = pl.multiple_of(i * (C // 2), C // 2)
            kw = kbuf.bitcast(U32)
            p0, p1, p2 = (kw[tf, pl.ds(h0 + 8 - n, C // 2), :] for n in range(3))
            ke, ko = _unpack(p0, 0), _unpack(p0, 1)
            ke1, ko1 = _unpack(p1, 0), _unpack(p1, 1)
            ko2 = _unpack(p2, 1)
            vw = vbuf.bitcast(U32)[tf, pl.ds(h0, C // 2), :]
            w0, w1, w2, w3 = (taps[tf, j:j + 1, :] for j in range(4))
            env["kv"] = [((w0 * ke + w1 * ko1 + w2 * ke1 + w3 * ko2) * _unpack(vw, 0)).astype(BF),
                         ((w0 * ko + w1 * ke + w2 * ko1 + w3 * ke1) * _unpack(vw, 1)).astype(BF)]
            env["kt"] = [from_regs(zb[pl.ds(T_OFF + i * 16 + 8 * p, 8)]) for p in range(2)]

        def load_dft():
            n = 16 // order.count("F")
            fparts.append([from_regs(zb[pl.ds(F_OFF + 16 * p + len(fparts) * n, n)]) for p in range(2)])

        def forward():
            fm = [jnp.concatenate([f[p] for f in fparts], axis=0) for p in range(2)]
            skip = jnp.where(i == 0, jnp.broadcast_to(taps[tf, 4:5, :], (8, LANES)), 0.0)
            for dst, x, lag0 in (((xs0, xs1)[tf % 2], env["kv"], None), ((ks0, ks1)[tf % 2], env["kt"], skip)):
                e, o = _dot(fm[0], x[0]), _dot(fm[1], x[1])
                for j in range(NPOS):
                    re, im = slice(16 * j, 16 * j + 8), slice(16 * j + 8, 16 * j + 16)
                    er = e[re] if lag0 is None else e[re] + lag0
                    dst[j, 0, 0, i], dst[j, 0, 1, i] = er + o[re], e[im] + o[im]
                    dst[j, 1, 0, i], dst[j, 1, 1, i] = er - o[re], e[im] - o[im]

        def product():
            xs, ks = (xs0, xs1)[ts % 2], (ks0, ks1)[ts % 2]
            half, f1, m = pieces.pop(0)
            j = i + half * (NPOS // 2)

            def operand(ref):
                if m < 2:
                    return [ref[j, f1, m, c] for c in range(NB)]
                return [ref[j, f1, 0, c] + ref[j, f1, 1, c] for c in range(NB)]
            x, k = operand(xs), operand(ks)
            for c, z in enumerate(_causal_conv(x, k)):
                zb[(ts * NB + c) * Z_CHUNK + j * 6 + f1 * 3 + m] = z

        def taps_ahead():
            transpose_taps(jnp.minimum(tf * NB + i + NB // 2, NT * NB - 1))

        ops = {"t": (tf, taps_ahead), "k": (tf, short_conv), "F": (tf, load_dft),
               "X": (tf, forward), "b": (ts, product)}
        for ch in order:
            tile, fn = ops[ch]
            if tile is not None:
                fn()

    def stage(t, events):
        def step(i, _):
            for at, fn in events.items():
                pl.when(i == at)(fn)
            for u in range(2):
                conv_step(2 * i + u, t, t - 1 if t else None, STEP_ORDER[u])
            return 0
        lax.fori_loop(0, NB // 2, step, 0)

    def inverse(b, t):
        base = (t * NB + b) * Z_CHUNK

        def position(j):
            z = []
            for f1 in range(2):
                p, q, r = (zb[base + j * 6 + f1 * 3 + m] for m in range(3))
                z.append((p - q, r - p - q))
            out = []
            for p, op in enumerate((jnp.add, jnp.subtract)):
                re, im = op(z[0][0], z[1][0]), op(z[0][1], z[1][1])
                if isinstance(b, int) and b == 0:
                    out.append((re, im))
                elif NPOS // 4 <= j < 3 * NPOS // 4:
                    out.append((re + carry[t, j, p, 1], im - carry[t, j, p, 0]))
                else:
                    out.append((re - carry[t, j, p, 1], im + carry[t, j, p, 0]))
                carry[t, j, p, 0], carry[t, j, p, 1] = re, im
            return out

        w = [[], [], [], []]
        for j in range(NPOS // 2):
            (r0, i0), (r1, i1) = position(j)
            (x0, y0), (x1, y1) = position(j + NPOS // 2)
            for p, (re, im) in enumerate(((r0 + x0, i0 - y0), (r1 - y1, i1 - x1),
                                          (r0 - x0, i0 + y0), (r1 + y1, i1 + x1))):
                w[p].append(_pack(re, im))
        y = [_dot(pltpu.bitcast(gm_ref[p], BF), pltpu.bitcast(jnp.concatenate(w[p], axis=0), BF))
             for p in range(4)]
        ybuf[t, pl.ds(0, C // 4, stride=2), :] = _pack(y[0], y[1])
        ybuf[t, pl.ds(1, C // 4, stride=2), :] = _pack(y[2], y[3])

    def pre(b, r, n):
        sa, ca1, ga, sb, cb1 = (jnp.concatenate([mod[:, j * D:(j + 1) * D]] * (n // 8), axis=0)
                                for j in range(5))
        x = qbuf[pl.ds(pl.multiple_of(b * C + r, n), n), :].astype(F32)
        y = jnp.concatenate([pltpu.bitcast(ybuf[t, r // 2:(r + n) // 2, :], BF) for t in range(NT)], axis=1)
        h = _layernorm(x) * ca1 + sa
        x1 = x + ga * (h * y.astype(F32))
        x1buf[b % 2, r:r + n, :] = x1
        h2 = pltpu.bitcast((_layernorm(x1) * cb1 + sb).astype(BF), U32)
        for t in range(NT):
            h2buf[b % 2, t, r // 2:(r + n) // 2, :] = h2[:, t * LANES:(t + 1) * LANES]
        return h2[n // 2 - 8:n // 2, 0:LANES]

    def cond():
        return jnp.broadcast_to(_silu(c_ref[...].astype(F32)), (16, D)).astype(BF)

    def mod_part(j):
        part = _dot(cond()[:, j * LANES:(j + 1) * LANES], wmbuf[j])[0:8]
        if j == 0:
            mod[...] = part
            for scale in (1, 4):
                mod[:, scale * D:(scale + 1) * D] = 1 + part[:, scale * D:(scale + 1) * D]
        else:
            mod[...] = mod[...] + part

    def mlp(b, zero, last=False, before=None):
        def matmul(x, wbuf, j, fill):
            cols = []
            for n, piece in enumerate(fill):
                cols.append(wbuf[j, :, n * LANES:(n + 1) * LANES])
                if piece and not last:
                    done = pre(b + 1, int(piece) * (C // NPRE), C // NPRE)
                    wbuf[NFC + zero, 0:16, 0:LANES] = pltpu.bitcast(done, BF)
            out = _dot(x, jnp.concatenate(cols, axis=1))
            if not last:
                for buf in (w1buf, w3buf, w2buf):
                    buf[NFC + zero, 16:32, 0:LANES] = pltpu.bitcast(out[0:8, 0:LANES], BF)
                zb[Z_ROWS - 1 + zero] = out[0:8, 0:LANES]
            return out

        h2 = jnp.concatenate([pltpu.bitcast(h2buf[b % 2, t], BF) for t in range(NT)], axis=1)
        g, a, acc = {}, {}, None
        for kind, j, *fill in BLOCK_ORDER:
            if kind == "I":
                if not last and not before:
                    inverse(b + 1, j)
                continue
            if before and kind + str(j) in before:
                before[kind + str(j)]()
            if kind == "g":
                g[j] = matmul(h2, w1buf, j, fill[0])
            elif kind == "u":
                a[j] = (_silu(g[j]) * matmul(h2, w3buf, j, fill[0])).astype(BF)
            else:
                p = matmul(a[j], w2buf, j, fill[0])
                acc = p if acc is None else acc + p
        gb = jnp.concatenate([gate[...]] * (C // 8), axis=0)
        res = (x1buf[b % 2] + gb * acc).astype(BF)
        if last:
            for t in range(NT):
                obuf[block_rows(b), lanes(t)] = res[:, t * LANES:(t + 1) * LANES]
                tail_copy(t).start()
        else:
            obuf[block_rows(b), :] = res
            start(o_copy(b))

    small = [pltpu.make_async_copy(src, dst, sem_small) for src, dst in (
        (shift_hbm, shift_ref), (d_hbm, d_ref), (c_hbm, c_ref), (gm_hbm, gm_ref),
        (fm_hbm, zb.at[pl.ds(F_OFF, 32)]))]
    start(s_copy(0) + small + k_copy(0))
    kbuf[:, 0:16, :] = jnp.zeros((NT, 16, LANES), BF)
    wait(s_copy(0))
    start(v_copy(0))
    for n in range(NB // 2):
        transpose_taps(n)
    wait(small)
    sh = shift_ref[...].astype(F32)
    dd = d_ref[...].astype(F32).reshape(1, D)
    for t in range(NT):
        taps[t, 0:4, :] = sh[:, t * LANES:(t + 1) * LANES]
        taps[t, 4:5, :] = dd[:, t * LANES:(t + 1) * LANES]
    wait(k_copy(0))
    start(s_copy(1))
    queue = [lambda t=t, copy=copy: copy(t) for t in range(1, NT) for copy in (s_copy, k_copy, v_copy)][1:]
    queue += [lambda j=j: wm_copy(j) for j in range(4)]
    issue = dict(zip(ISSUE_AT, queue))
    for t in range(NT):
        def event(i, t=t):
            def fn():
                if t * NB // 2 + i in issue:
                    start(issue[t * NB // 2 + i]())
                if i == NB // 4 and t + 1 < NT:
                    wait(s_copy(t + 1))
            return fn
        wait((k_copy(t) if t else []) + v_copy(t))
        stage(t, {i: event(i) for i in range(NB // 2)})
    start(wm_copy(4))
    for i in range(NB):
        if i == 2:
            wait(wm_copy(0) + wm_copy(1) + wm_copy(2))
            start(q_copy(0) + w1_copy(0))
        if i == 6:
            wait(wm_copy(3) + wm_copy(4))
            start(w3_copy(0))
        if i in (2, 3, 4, 6, 7):
            mod_part((2, 3, 4, 6, 7).index(i))
        if i < NT - 1:
            inverse(0, i)
        conv_step(i, None, NT - 1)
    inverse(0, NT - 1)
    wait(q_copy(0))
    pre(0, 0, C)
    start(w2_copy(0) + q_copy(1))
    for t in range(NT):
        inverse(1, t)

    def arrive(copies, then):
        def fn():
            wait(copies())
            start(then())
        return fn

    def gate_out():
        wait(w2_copy(2) + gate_copy())
        start([cp for b in range(2, NB) for cp in q_copy(b)])
        gate[...] = _dot(cond(), wgbuf[...])[0:8]

    mlp(0, pl.program_id(0), before={
        "g0": arrive(lambda: w1_copy(0) + w3_copy(0), lambda: w1_copy(1) + w3_copy(1)),
        "d0": arrive(lambda: w2_copy(0) + q_copy(1) + w1_copy(1), lambda: w2_copy(1) + w1_copy(2)),
        "u1": arrive(lambda: w3_copy(1) + w2_copy(1), lambda: w3_copy(2) + w2_copy(2) + gate_copy()),
        "g2": arrive(lambda: w1_copy(2) + w3_copy(2), lambda: []),
        "d2": gate_out})

    def middle(i, _):
        wait(q_copy(i + 2))
        mlp(i + 1, i // NB)
        return 0

    lax.fori_loop(0, NB - 2, middle, 0)
    mlp(NB - 1, 0, last=True)
    for b in range(NB - 1):
        wait(o_copy(b))
    wait([tail_copy(t) for t in range(NT)])


@jax.jit
def pallas_adaLN_cond__ssm_conv_h3__glu_gated_swiglu__prompt_kernel(
        A_q, A_k, A_v, A_shift_k, A_ssm_k, A_ssm_D, B_x, B_w1, B_w3, B_w2, c, w_mod):
    del B_x
    fm, gm = _dft_consts()
    any_spec = pl.BlockSpec(memory_space=pl.ANY)
    spectrum = pltpu.VMEM((NPOS, 2, 2, NB, 8, LANES), F32)
    return pl.pallas_call(
        _body,
        grid=(1,),
        out_shape=jax.ShapeDtypeStruct((1, S, D), BF),
        in_specs=[any_spec] * 13,
        out_specs=any_spec,
        scratch_shapes=[
            pltpu.VMEM((4, D), BF),
            pltpu.VMEM((D,), BF),
            pltpu.VMEM((1, D), BF),
            pltpu.VMEM((4, 32, LANES), U32),
            pltpu.VMEM((NT, S + 16, LANES), BF),
            pltpu.VMEM((NT, S, LANES), BF),
            pltpu.VMEM((NT, LANES, S), BF),
            pltpu.VMEM((S, D), BF),
            pltpu.VMEM((NFC + 1, D, FC), BF),
            pltpu.VMEM((NFC + 1, D, FC), BF),
            pltpu.VMEM((NFC + 1, FC, D), BF),
            pltpu.VMEM((NT, LANES, 5 * D), BF),
            pltpu.VMEM((D, D), BF),
            pltpu.VMEM((NT, C // 2, LANES), U32),
            pltpu.VMEM((S, D), BF),
            spectrum, spectrum, spectrum, spectrum,
            pltpu.VMEM((Z_ROWS, 8, LANES), F32),
            pltpu.VMEM((NT, NPOS, 2, 2, 8, LANES), F32),
            pltpu.VMEM((NT, 8, LANES), F32),
            pltpu.VMEM((8, 5 * D), F32),
            pltpu.VMEM((8, D), F32),
            pltpu.VMEM((2, C, D), F32),
            pltpu.VMEM((2, NT, C // 2, LANES), U32),
            pltpu.SemaphoreType.DMA((3, NT)),
            pltpu.SemaphoreType.DMA((6,)),
            pltpu.SemaphoreType.DMA((NB,)),
            pltpu.SemaphoreType.DMA((3, NFC)),
            pltpu.SemaphoreType.DMA((NB,)),
            pltpu.SemaphoreType.DMA(()),
        ],
        compiler_params=pltpu.CompilerParams(vmem_limit_bytes=100 * 2**20),
    )(A_q, A_k, A_v, A_shift_k.T, A_ssm_k, A_ssm_D, B_w1, B_w3, B_w2, c, w_mod,
      jnp.asarray(fm), jnp.asarray(gm))
```
